```python
import os as _os
_os.environ.setdefault("JAX_PLATFORMS", "cpu")
import jax
import jax.numpy as jnp

def _softmax(x, axis=-1):
    return jax.nn.softmax(x, axis=axis)
def _gelu(x):
    return jax.nn.gelu(x, approximate=True)
def _silu(x):
    return jax.nn.silu(x)
def _sigmoid(x):
    return jax.nn.sigmoid(x)
def _layernorm(x, axis=-1, eps=1e-5):
    m = jnp.mean(x, axis=axis, keepdims=True)
    v = jnp.var(x, axis=axis, keepdims=True)
    return (x - m) / jnp.sqrt(v + eps)
def _scatter_add(tgt, idx, src, axis=0):
    return tgt.at[idx].add(src)
def _segment_sum(src, seg, n):
    return jax.ops.segment_sum(src, seg, n)
class _Rng:
    def __init__(self, key):
        self._k = key
    def _next(self):
        self._k, sub = jax.random.split(self._k)
        return sub
    def normal(self, shape):
        return jax.random.normal(self._next(), shape, dtype=jnp.bfloat16)
    def randint(self, lo, hi, shape):
        return jax.random.randint(self._next(), shape, lo, hi, dtype=jnp.int32)
    def uniform(self, shape, lo=0.0, hi=1.0):
        return jax.random.uniform(self._next(), shape, jnp.bfloat16, lo, hi)
    def permutation(self, n):
        return jax.random.permutation(self._next(), n)


kernel_name = 'parallel_sum__mha_block__dense_activation_mish__prompt'

def setup_inputs():
    _rng = _Rng(jax.random.key(int.from_bytes(__import__("os").urandom(4), "little")))
    _w = (lambda a: (lambda t: t.astype(jnp.bfloat16) if jnp.issubdtype(t.dtype, jnp.floating) else t)(jnp.asarray(a)))
    def _A_setup():
        B, S, D, H = 1, 2048, 512, 32
        return {
            "x": _w((lambda *s: _rng.normal(s) * 0.05)(B, S, D)),
            "wqkv": _w((lambda *s: _rng.normal(s) * 0.05)(D, 3 * D)),
            "wo": _w((lambda *s: _rng.normal(s) * 0.05)(D, D)),
        }
    _A_in = _A_setup()

    def _B_setup():
        B, S, D, F = 1, 2048, 512, 1792
        return {
            "x": _w((lambda *s: _rng.normal(s) * 0.05)(B, S, D)),
            "w1": _w((lambda *s: _rng.normal(s) * 1.6)(D, F) * (D ** -0.5)),
            "b1": _w((lambda *s: _rng.normal(s) * 0.05)(F)),
            "w2": _w((lambda *s: _rng.normal(s) * 0.05)(F, D) * (F ** -0.5)),
        }
    _B_in = _B_setup()

    return {
        "A_x": _A_in["x"],
        "A_wqkv": _A_in["wqkv"],
        "A_wo": _A_in["wo"],
        "B_x": _B_in["x"],
        "B_w1": _B_in["w1"],
        "B_b1": _B_in["b1"],
        "B_w2": _B_in["w2"],
    }

def reference(A_x, A_wqkv, A_wo, B_x, B_w1, B_b1, B_w2):
    def _A_ref(x, wqkv, wo):
        B, S, D = x.shape
        H = 32
        Dh = D // H
        qkv = (lambda x, *d: x.transpose(*d))((x @ wqkv).reshape(B, S, 3, H, Dh), 2, 0, 3, 1, 4)
        q, k, v = qkv[0], qkv[1], qkv[2]
        scores = jnp.einsum("bhqd,bhkd->bhqk", q, k) * (Dh ** -0.5)
        p = _softmax(scores, axis=-1)
        o = jnp.einsum("bhqk,bhkd->bhqd", p, v)
        return (lambda x, *d: x.transpose(*d))(o, 0, 2, 1, 3).reshape(B, S, D) @ wo

    def _B_ref(x, w1, b1, w2):
        h = jnp.einsum("bsd,df->bsf", x, w1) + b1
        sp = jnp.log1p(jnp.exp(-jnp.abs(h))) + jnp.where(h > 0, h, jnp.zeros_like(h))
        act = h * jnp.tanh(sp)
        return jnp.einsum("bsf,fd->bsd", act, w2)

    x = A_x
    xn = _layernorm(x, axis=-1)
    return x + _A_ref(xn, A_wqkv, A_wo) + _B_ref(xn, B_w1, B_b1, B_w2)
```

```python
import functools

import jax
import jax.numpy as jnp
import numpy as np
from jax import lax
from jax.experimental import pallas as pl
from jax.experimental.pallas import tpu as pltpu

F32, BF16, U32 = jnp.float32, jnp.bfloat16, jnp.uint32
LOG2E = float(np.log2(np.e))
H, DH = 32, 16
TQ = 512
TK = 128
NT = TQ // 128
L_LO, L_HI = 2.0 ** -40, 2.0 ** 40


def _pack(x):
    return pltpu.bitcast(x.astype(BF16), U32)


def _unpack(x):
    return pltpu.bitcast(x, BF16)


def _mish(h):
    e = jnp.exp2(jnp.minimum(h * LOG2E, 30.0))
    n = e * (e + 2.0)
    return h * (n * pl.reciprocal(n + 2.0, approx=True))


def make(R=384, G=2, T=1, pfmt="u32", glag=3, flags=None, name="fused", vlead=0.0, plag=0, ffn=True, dbg='', kbg=4, dstart=0, dend=0):
    def kernel(x_hbm, wqkv_hbm, wo_hbm, w1_hbm, b1_ref, w2_hbm, out_hbm,
               x_v, wk_v, wqv_v, wo_v, w1_v, w2_v, w1_s, w2_s, wqvt_s, b1_s, xn_s, k_s, kf_s, qt_s, vt_s,
               qp_s, oc_s, l_s, pa_s, pb_s, ot_s, acc_s, out_v, sems):
        S, D = x_v.shape
        NF = w1_v.shape[0]
        NQB = S // TQ
        NKC = S // TK
        SH = S // 2
        RH = R // 2
        NG = RH // 8
        RB = 256
        NRB = S // RB

        def x_cp(i):
            return pltpu.make_async_copy(x_hbm.at[0, pl.ds(i * RB, RB), :], x_v.at[pl.ds(i * RB, RB), :], sems.at[i])

        def col_cp(src, col, dst, sem):
            return pltpu.make_async_copy(src.at[:, pl.ds(col, 128)], dst, sems.at[sem])

        wk_cps = [col_cp(wqkv_hbm, D + 128 * c, wk_v.at[c], NRB) for c in range(4)]
        wqv_cps = [col_cp(wqkv_hbm, (0 if c < 4 else D) + 128 * c, wqv_v.at[c], NRB + 1) for c in range(8)]
        w1_cps = [col_cp(w1_hbm, 128 * c, w1_v.at[c], NRB + 2) for c in range(NF)]
        w2_cps = [col_cp(w2_hbm, 128 * c, w2_v.at[c], NRB + 3) for c in range(4)]
        wo_cps = [col_cp(wo_hbm, 128 * c, wo_v.at[c], NRB + 4) for c in range(4)]
        x_cp(0).start()
        for c in wk_cps:
            c.start()
        for i in range(1, NRB):
            x_cp(i).start()
        for c in wqv_cps + w1_cps + w2_cps + wo_cps:
            c.start()

        pb_s[pl.ds(0, pb_s.shape[0] - R * 2), :] = jnp.zeros((pb_s.shape[0] - R * 2, TQ), pb_s.dtype)
        qp_s[...] = jnp.zeros(qp_s.shape, U32)
        oc_s[...] = jnp.zeros(oc_s.shape, F32)
        l_s[...] = jnp.full(l_s.shape, 0.125, F32)
        b1 = b1_ref[...].astype(F32)
        for c in range(NF):
            b1_s[c] = jnp.broadcast_to(b1[c:c + 1, :], (8, 128))

        for c in wk_cps:
            c.wait()

        def layernorm(i):
            x = x_v[pl.ds(i * RB, RB), :].astype(F32)
            xc = x - jnp.mean(x, axis=-1, keepdims=True)
            var = jnp.mean(xc * xc, axis=-1, keepdims=True)
            xn_s[pl.ds(i * RB // 2, RB // 2), :] = _pack(xc * lax.rsqrt(var + 1e-5))

        def k_proj(i):
            xn = _unpack(xn_s[pl.ds(i * RB // 2, RB // 2), :])
            wk = jnp.concatenate([wk_v[c] for c in range(4)], axis=1)
            k = jnp.dot(xn, wk, preferred_element_type=F32)
            kp = _pack(k)
            for c in range(4):
                k_s[c, pl.ds(i * RB // 2, RB // 2), :] = kp[:, c * 128:(c + 1) * 128]
            kh = i * RB // SH
            v0 = (kh + 1) * SH - RH
            lo = max(i * RB, v0)
            if lo < (i + 1) * RB:
                for c in range(4):
                    kf_s[c, kh, pl.ds(lo - v0, (i + 1) * RB - lo), :] = k[lo - i * RB:, c * 128:(c + 1) * 128]

        x_cp(0).wait()
        layernorm(0)
        for i in range(NRB):
            if i + 1 < NRB:
                x_cp(i + 1).wait()
                layernorm(i + 1)
            if i == NRB - 2:
                for c in wqv_cps:
                    c.wait()
                for c in range(8):
                    wqvt_s[pl.ds(c * 64, 64), :] = _pack(wqv_v[c].astype(F32).T)
            k_proj(i)

        PR = SH // 2 if pfmt == "u32" else SH

        def kb_slot(d, g, base=None):
            i = d * NG + g
            row = 2 * PR + (i // NT) * 8
            if base is not None:
                row = pl.multiple_of(base + row, 8)
            return pl.ds(row, 8), pl.ds((i % NT) * 128, 128)

        def kb_prep(dst, h, kh, d, groups, base=None):
            idx = jnp.full((8, 128), (h % 8) * DH + d, jnp.int32)
            for g in groups:
                kb = jnp.take_along_axis(kf_s[h // 8, kh, pl.ds(g * 8, 8), :], idx, axis=1)
                dst[kb_slot(d, g, base)] = pltpu.bitcast(kb, dst.dtype)

        for qb in range(NQB):
            xn = _unpack(xn_s[pl.ds(qb * TQ // 2, TQ // 2), :])
            qv = lax.dot_general(_unpack(wqvt_s[...]), xn, (((1,), (1,)), ((), ())), preferred_element_type=F32)
            q = qv[:D] * (DH ** -0.5 * LOG2E)
            v = qv[D:]
            vp = _pack(v) if pfmt == "u32" else v
            vr = vp.shape[0] // H
            for h in range(H):
                qt_s[h, qb] = q[h * DH:(h + 1) * DH]
                for t in range(NT):
                    vt_s[h, qb * NT + t] = vp[h * vr:(h + 1) * vr, t * 128:(t + 1) * 128]
            if qb == 0:
                for d in range(DH):
                    kb_prep(pb_s, 0, 0, d, range(NG))
            if qb == NQB - 2:
                for c in w1_cps + w2_cps:
                    c.wait()
                for c in range(NF):
                    w1_s[c] = pltpu.bitcast(w1_v[c], U32)
                for c in range(4):
                    w2_s[:, pl.ds(c * 128, 128)] = pltpu.bitcast(w2_v[c], U32)

        NKH = SH // TK
        nm = (SH - RH) // 16
        m_cut = [(nm * j) // NKH for j in range(NKH + 1)]
        v_pieces = [(u, b, t) for u in range(2) for b in range(RH // (8 * G)) for t in range(0, NT, T)]
        k_pieces = [(d, g) for d in range(DH) for g in range(0, NG, kbg)] if 'nokb' not in dbg else []
        events = sorted([((a + 0.5) / (2 * nm), 0, a) for a in range(2 * nm)]
                        + [((i + 0.5 - vlead) / len(v_pieces), 1, i) for i in range(len(v_pieces))]
                        + [((i + 0.5) / len(k_pieces), 2, i) for i in range(len(k_pieces))])
        FR = S // (2 * H)
        dense = {}
        if ffn:
            order = [("g1", c) for c in range(NF)]
            for c in range(NF):
                order.insert(min(2 * c + glag - 1, len(order)), ("g2", c))
            for i, op in enumerate(order):
                dense.setdefault(dstart + (i * (2 * NKC - dstart - dend)) // len(order), []).append(op)

        def load_p(p_ref, u, j):
            if pfmt == "u32":
                return _unpack(p_ref[pl.ds(u * PR + j * TK // 2, TK // 2), :])
            return p_ref[pl.ds(u * PR + j * TK, TK), :]

        def load_v(h, j):
            return _unpack(vt_s[h, j]) if pfmt == "u32" else vt_s[h, j]

        def attn_step(h, qh, kh, l, p_wr, p_rd, h_next, zero, pv_dot, side_work):
            q_off = pl.multiple_of((7 - h % 8) * 8, 8)

            def add_l(u, t, p):
                for g in range(p.shape[0] // 8):
                    y = p[g * 8:(g + 1) * 8]
                    l[u][t] = y if l[u][t] is None else l[u][t] + y

            def store_p(u, row, t, p, base):
                if pfmt == "u32":
                    p, row = _pack(p), row // 2
                row += u * PR
                if base is not None:
                    row = pl.multiple_of(base + row, 8)
                p_wr[pl.ds(row, p.shape[0]), pl.ds(t * 128, p.shape[1])] = p

            def mxu_piece(s, u, a, a0):
                p = jnp.exp2(s[(a - a0) * 16:(a - a0 + 1) * 16])
                for t in range(NT):
                    add_l(u, t, p[:, t * 128:(t + 1) * 128])
                store_p(u, a * 16, 0, p, None)

            def vpu_piece(u, b, t0):
                sv = [[None] * T for _ in range(G)]
                for d in range(DH):
                    kb = [pltpu.bitcast(p_rd[kb_slot(d, G * b + g)], F32) for g in range(G)]
                    for t in range(T):
                        qd = jnp.broadcast_to(qt_s[h, 2 * qh + u, pl.ds(d, 1), pl.ds((t0 + t) * 128, 128)], (8, 128))
                        for g in range(G):
                            pr = kb[g] * qd
                            sv[g][t] = pr if d == 0 else sv[g][t] + pr
                for t in range(T):
                    p = jnp.exp2(jnp.concatenate([sv[g][t] for g in range(G)], axis=0))
                    add_l(u, t0 + t, p)
                    store_p(u, SH - RH + b * 8 * G, t0 + t, p, zero)

            ev = 0
            for u in range(2):
                for j in range(NKH):
                    a0, a1 = m_cut[j], m_cut[j + 1]
                    s = jnp.dot(_unpack(k_s[h // 8, pl.ds(kh * SH // 2 + a0 * 8, (a1 - a0) * 8), :]),
                                _unpack(qp_s[pl.ds(q_off, 64), pl.ds(u * TQ, TQ)]), preferred_element_type=F32)
                    while ev < len(events) and (events[ev][1] or events[ev][2] < u * nm + a1):
                        _, kind, i = events[ev]
                        ev += 1
                        if kind == 0:
                            mxu_piece(s, u, i - u * nm, a0)
                        elif kind == 1:
                            vpu_piece(*v_pieces[i])
                        else:
                            d, g = k_pieces[i]
                            kb_prep(p_wr, h_next, 1 - kh, d, range(g, min(g + kbg, NG)), zero)
                    period = (2 * kh + u) * NKH + j
                    pv_dot(period - kh * plag)
                    side_work(period)

        def inv_l(u, l_min, l_max):
            l = jnp.sum(l_s[u], axis=0, keepdims=True)
            r = pl.reciprocal(l, approx=True)
            return r * (2.0 - l * r), jnp.minimum(l_min, l), jnp.maximum(l_max, l)

        def body(it, carry):
            l_min, l_max = carry
            h, qh = it // 2, it % 2
            itp, itn = jnp.maximum(it - 1, 0), jnp.minimum(it + 1, 2 * H - 1)
            zero = (it // (2 * H)) * 16
            st = {"pv": -1}
            xn_row = pl.multiple_of(it * (FR // 2), 8)
            inv = []
            for u in range(2):
                r, l_min, l_max = inv_l(u, l_min, l_max)
                inv.append(r)
                qp_s[pl.ds(56, 8), pl.ds(u * TQ, TQ)] = _pack(qt_s[h, 2 * qh + u])

            def pv_dot(period):
                if period <= st["pv"]:
                    return
                st["pv"] = period
                kh, u, j = period // NKC, period // NKH % 2, period % NKH
                if kh == 0:
                    pv = jnp.dot(load_v(itp // 2, NKH + j), load_p(pb_s, u, j), preferred_element_type=F32)
                    st["o"] = (oc_s[u] if j == 0 else st["o"]) + pv
                    if j == NKH - 1:
                        ot_s[itp // 2, 2 * (itp % 2) + u] = _pack(st["o"] * inv[u])
                else:
                    pv = jnp.dot(load_v(h, j), load_p(pa_s, u, j), preferred_element_type=F32)
                    st["o"] = pv if j == 0 else st["o"] + pv
                    if j == NKH - 1:
                        oc_s[u] = st["o"]

            def side_work(period):
                for kind, c in dense.get(period, ()):
                    if kind == "g1":
                        hid = jnp.dot(_unpack(xn_s[pl.ds(xn_row, FR // 2), :]), _unpack(w1_s[c]), preferred_element_type=F32)
                        st[c] = _mish(hid + jnp.concatenate([b1_s[c]] * (FR // 8), axis=0)).astype(BF16)
                    else:
                        y = jnp.dot(st.pop(c), _unpack(w2_s[pl.ds(c * 64, 64), :]), preferred_element_type=F32)
                        st["acc"] = y if c == 0 else st["acc"] + y

            l = [[None] * NT for _ in range(2)]
            attn_step(h, qh, 0, l, pa_s, pb_s, h, zero, pv_dot, side_work)
            attn_step(h, qh, 1, l, pb_s, pa_s, itn // 2, zero, pv_dot, side_work)
            for period in range(2 * NKC - plag, 2 * NKC):
                pv_dot(period)
            for u in range(2):
                l_s[u] = jnp.concatenate(l[u], axis=1)
            if ffn:
                acc_s[pl.ds(pl.multiple_of(it * FR, 8), FR), :] = st["acc"]
            return l_min, l_max

        one = jnp.ones((1, TQ), F32)
        l_min, l_max = lax.fori_loop(0, 2 * H, body, (one, one))
        v_last = jnp.concatenate([load_v(H - 1, NKH + j) for j in range(NKH)], axis=1)
        for u in range(2):
            p_last = jnp.concatenate([load_p(pb_s, u, j) for j in range(NKH)], axis=0)
            r, l_min, l_max = inv_l(u, l_min, l_max)
            ot_s[H - 1, 2 + u] = _pack((oc_s[u] + jnp.dot(v_last, p_last, preferred_element_type=F32)) * r)

        ok = jnp.where((l_min >= L_LO) & (l_max <= L_HI), 1.0, 0.0)

        @pl.when(jnp.min(ok) < 0.5)
        def _():
            def safe_step(i, carry):
                h, qb = i // NQB, i % NQB
                qp_s[pl.ds(56, 8), pl.ds(0, TQ)] = _pack(qt_s[h, qb])
                qm = _unpack(qp_s[pl.ds(pl.multiple_of((7 - h % 8) * 8, 8), 64), pl.ds(0, TQ)])

                def scores(j):
                    return jnp.dot(_unpack(k_s[h // 8, pl.ds(pl.multiple_of(j * (TK // 2), 8), TK // 2), :]), qm,
                                   preferred_element_type=F32)

                m = lax.fori_loop(0, NKC, lambda j, m: jnp.maximum(m, jnp.max(scores(j), axis=0, keepdims=True)),
                                  jnp.full((1, TQ), -jnp.inf, F32))

                def accumulate(j, c):
                    p = jnp.exp2(scores(j) - m)
                    pm = p.astype(BF16) if pfmt == "u32" else p
                    return (c[0] + jnp.sum(p, axis=0, keepdims=True),
                            c[1] + jnp.dot(load_v(h, j), pm, preferred_element_type=F32))

                l, o = lax.fori_loop(0, NKC, accumulate, (jnp.zeros((1, TQ), F32), jnp.zeros((DH, TQ), F32)))
                ot_s[h, qb] = _pack(o / l)
                return carry

            lax.fori_loop(0, H * NQB, safe_step, 0)

        for c in wo_cps:
            c.wait()

        def out_cp(i):
            return pltpu.make_async_copy(out_v.at[pl.ds(i * RB, RB), :], out_hbm.at[0, pl.ds(i * RB, RB), :], sems.at[i])

        for i in range(NRB):
            qb, c0 = i * RB // TQ, i * RB % TQ
            ot = _unpack(jnp.concatenate([ot_s[h, qb, :, pl.ds(c0, RB)] for h in range(H)], axis=0))
            wo = jnp.concatenate([wo_v[c] for c in range(4)], axis=1)
            y = lax.dot_general(ot, wo, (((0,), (0,)), ((), ())), preferred_element_type=F32)
            rows = pl.ds(i * RB, RB)
            res = x_v[rows, :].astype(F32) + y
            if ffn:
                res = res + acc_s[rows, :]
            out_v[rows, :] = res.astype(out_v.dtype)
            out_cp(i).start()
        for i in range(NRB):
            out_cp(i).wait()

    def call(A_x, A_wqkv, A_wo, B_x, B_w1, B_b1, B_w2):
        del B_x
        _, S, D = A_x.shape
        F = B_w1.shape[1]
        NF = F // 128
        NG = max(R // 16, 1)
        vm = pltpu.VMEM
        p_shape = vm((S // 2 + R * 2, TQ), U32) if pfmt == "u32" else vm((S + R * 2, TQ), F32)
        any_spec = pl.BlockSpec(memory_space=pl.ANY)
        return pl.pallas_call(
            kernel,
            out_shape=jax.ShapeDtypeStruct(A_x.shape, A_x.dtype),
            in_specs=[any_spec, any_spec, any_spec, any_spec, pl.BlockSpec(memory_space=pltpu.VMEM), any_spec],
            out_specs=any_spec,
            scratch_shapes=[
                vm((S, D), BF16),
                vm((4, D, 128), BF16),
                vm((8, D, 128), BF16),
                vm((4, D, 128), BF16),
                vm((NF, D, 128), BF16),
                vm((4, F, 128), BF16),
                vm((NF, D // 2, 128), U32),
                vm((F // 2, D), U32),
                vm((D, D), U32),
                vm((-(-NF // 8) * 8, 8, 128), F32),
                vm((S // 2, D), U32),
                vm((4, S // 2, 128), U32),
                vm((4, 2, -(-NG // 8) * 64, 128), F32),
                vm((H, S // TQ, DH, TQ), F32),
                vm((H, S // TK, 8, TK), U32) if pfmt == "u32" else vm((H, S // TK, DH, TK), F32),
                vm((120, 2 * TQ), U32),
                vm((2, DH, TQ), F32),
                vm((2, 8, TQ), F32),
                p_shape, p_shape,
                vm((H, S // TQ, 8, TQ), U32),
                vm((S, D), F32),
                vm((S, D), BF16),
                pltpu.SemaphoreType.DMA((16,)),
            ],
            compiler_params=pltpu.CompilerParams(vmem_limit_bytes=100 << 20, flags=flags),
            name=name,
        )(A_x, A_wqkv, A_wo, B_w1, B_b1.reshape(NF, 128), B_w2)

    return call


@jax.jit
def pallas_parallel_sum__mha_block__dense_activation_mish__prompt_kernel(
    A_x: jax.Array,
    A_wqkv: jax.Array,
    A_wo: jax.Array,
    B_x: jax.Array,
    B_w1: jax.Array,
    B_b1: jax.Array,
    B_w2: jax.Array,
):
    return make(R=256)(A_x, A_wqkv, A_wo, B_x, B_w1, B_b1, B_w2)
```

```python
import jax
import jax.numpy as jnp
import numpy as np
from jax import lax
from jax.experimental import pallas as pl
from jax.experimental.pallas import tpu as pltpu

F32, BF16, U32 = jnp.float32, jnp.bfloat16, jnp.uint32
LOG2E = float(np.log2(np.e))
H, DH = 32, 16
TQ = 512
TK = 128
NT = TQ // 128
L_LO, L_HI = 2.0 ** -40, 2.0 ** 40


def _pack(x):
    return pltpu.bitcast(x.astype(BF16), U32)


def _unpack(x):
    return pltpu.bitcast(x, BF16)


def _mish(h):
    e = jnp.exp2(jnp.minimum(h * LOG2E, 30.0))
    n = e * (e + 2.0)
    return h * (n * pl.reciprocal(n + 2.0, approx=True))


def make(RU=((160,) * 4, (192,) * 4), vspan=((0, 1), (0.015, 1.03)), trun=(5, 6), kspan=0.97, kbg=6,
         plag=2, g1span=(1, 0), g2span=(0, 0), G1M=32, X0=512, R1=128, RB=256, name="fused", dbg=''):
    RS = [max(r) for r in RU]
    NGM = max(RS) // 8
    LO = 'looponly' in dbg

    def kernel(x_hbm, wqkv_hbm, wo_hbm, w1_hbm, b1_hbm, w2_hbm, out_hbm,
               x_v, wqkv_v, wo_v, w1_v, w2_v, w1_s, w2_s, b1_s, xn_s, k_s, kf_s, qt_s, vt_s, qp_s,
               kha_s, khb_s, act_s, oc_s, l_s, pa_s, pb_s, ot_s, acc_s, out_v, b1_v, sems):
        S, D = x_v.shape
        NF = w1_v.shape[1] // 128
        NQB = S // TQ
        SH = S // 2
        NKH = SH // TK
        NP = NQB * NKH
        PR = SH // 2
        FR = S // H
        kh_bufs = (kha_s, khb_s)

        def x_cp(r0, r1, sem):
            return pltpu.make_async_copy(x_hbm.at[0, pl.ds(r0, r1 - r0), :], x_v.at[pl.ds(r0, r1 - r0), :], sems.at[sem])

        def wqkv_cp(i):
            return pltpu.make_async_copy(wqkv_hbm.at[:, pl.ds(i * D, D)], wqkv_v.at[:, pl.ds(i * D, D)], sems.at[2 + i])

        late_cps = [pltpu.make_async_copy(src, dst, sems.at[5 + i])
                    for i, (src, dst) in enumerate(((w1_hbm, w1_v), (w2_hbm, w2_v), (wo_hbm, wo_v), (b1_hbm, b1_v)))]

        def kb_slot(d, g):
            i = g * DH + d
            return pl.ds(NQB * PR + (i // NT) * 8, 8), pl.ds((i % NT) * 128, 128)

        def kb_prep(dst, h, kh, d, groups):
            idx = jnp.full((8, 128), (h % 8) * DH + d, jnp.int32)
            for g in groups:
                kb = jnp.take_along_axis(kf_s[h // 8, kh, pl.ds(g * 8, 8), :], idx, axis=1, mode="promise_in_bounds")
                dst[kb_slot(d, g)] = pltpu.bitcast(kb, U32)

        def kh_prep(h, kh):
            n = (SH - min(RU[kh])) // 2
            k = k_s[h // 8, pl.ds(kh * SH // 2, n), :]
            kh_bufs[kh][pl.ds(0, n), :] = pltpu.roll(k, (128 - (h % 8) * DH) % 128, axis=1)

        def pv_dot(h, kh, p_ref, u, j):
            p = _unpack(p_ref[pl.ds(u * PR + j * TK // 2, TK // 2), :])
            return jnp.dot(_unpack(vt_s[h, kh * NKH + j]), p, preferred_element_type=F32)

        def inv_sum(u, l_min, l_max):
            l = jnp.sum(l_s[u], axis=0, keepdims=True)
            r = pl.reciprocal(l, approx=True)
            return r * (2.0 - l * r), jnp.minimum(l_min, l), jnp.maximum(l_max, l)

        def layernorm(r0, n):
            if LO and r0: return
            x = x_v[pl.ds(r0, n), :].astype(F32)
            xc = x - jnp.mean(x, axis=-1, keepdims=True)
            var = jnp.mean(xc * xc, axis=-1, keepdims=True)
            xn_s[pl.ds(r0 // 2, n // 2), :] = _pack(xc * lax.rsqrt(var + 1e-5))

        def project(r0, n, i):
            return jnp.dot(_unpack(xn_s[pl.ds(r0 // 2, n // 2), :]), wqkv_v[:, pl.ds(i * D, D)],
                           preferred_element_type=F32)

        def k_proj(r0, n):
            if LO and r0 != SH - RB: return
            k = project(r0, n, 1)
            kp = _pack(k)
            kh = r0 // SH
            v0 = (kh + 1) * SH - RS[kh]
            lo = max(r0, v0)
            for c in range(D // 128):
                k_s[c, pl.ds(r0 // 2, n // 2), :] = kp[:, c * 128:(c + 1) * 128]
                if lo < r0 + n:
                    kf_s[c, kh, pl.ds(lo - v0, r0 + n - lo), :] = k[lo - r0:, c * 128:(c + 1) * 128]

        def qv_proj(r0):
            if LO and r0: return
            q = (project(r0, RB, 0) * (DH ** -0.5 * LOG2E)).T
            v = project(r0, RB, 2).T
            u, cols = r0 // TQ, pl.ds(r0 % TQ, RB)
            for h in range(H):
                qt_s[h, u, :, cols] = q[h * DH:(h + 1) * DH]
                qp_s[h, u, :, cols] = _pack(q[h * DH:(h + 1) * DH])
                for t in range(RB // TK):
                    vt_s[h, r0 // TK + t] = _pack(v[h * DH:(h + 1) * DH, t * TK:(t + 1) * TK])

        x_cp(0, X0, 0).start()
        wqkv_cp(1).start()
        pb_s[pl.ds(0, NQB * PR), :] = jnp.zeros((NQB * PR, TQ), U32)
        oc_s[...] = jnp.zeros(oc_s.shape, F32)
        ot_s[H - 1] = jnp.zeros(ot_s.shape[1:], U32)
        l_s[...] = jnp.full(l_s.shape, 0.125, F32)
        wqkv_cp(0).start()
        x_cp(0, X0, 0).wait()
        wqkv_cp(1).wait()
        wqkv_cp(2).start()
        for r0 in range(0, X0, R1):
            layernorm(r0, R1)
            if r0 == X0 // 2:
                x_cp(X0, S, 1).start()
            k_proj(r0, R1)
        wqkv_cp(0).wait()
        wqkv_cp(2).wait()
        for r0 in range(0, X0 - RB, RB):
            qv_proj(r0)
        x_cp(X0, S, 1).wait()
        for c in late_cps:
            c.start()
        qv_proj(X0 - RB)
        for r0 in range(X0, S, RB):
            layernorm(r0, RB)
            if r0 + RB < S:
                k_proj(r0, RB)
        for d in range(DH):
            kb_prep(pb_s, 0, 0, d, range(RS[0] // 8))
        kh_prep(0, 0)
        for r0 in range(X0, S - RB, RB):
            qv_proj(r0)
        for c in late_cps:
            c.wait()
        qv_proj(S - RB)
        k_proj(S - RB, RB)
        for c in range(NF):
            w1_s[c] = pltpu.bitcast(w1_v[:, pl.ds(c * 128, 128)], U32)
        w2_s[...] = pltpu.bitcast(w2_v[...], U32)
        b1 = b1_v[...].astype(F32)
        for c in range(NF):
            b1_s[c] = jnp.broadcast_to(b1[c:c + 1, :], (8, 128))

        ffn_ops = ([(c, r) for c in range(NF) for r in range(0, FR, G1M)],
                   [op for n in (0, 2) for op in ((n, 0), (n, 4), (n, 8), (n, 12), (n + 1, 0), (n + 1, 4), (n + 1, 8))])
        ffn_at = [{lo + (i * (NP - lo - hi)) // len(ops): op for i, op in enumerate(ops)}
                  for ops, (lo, hi) in zip(ffn_ops, (g1span, g2span))]
        assert [len(a) for a in ffn_at] == [len(ops) for ops in ffn_ops]

        def score_step(h, kh, l, p_wr, p_rd, h_next, zero, pv_step, ffn_step):
            p_paced = p_wr.at[pl.ds(pl.multiple_of(zero, 16), p_wr.shape[0])]
            kh_prep(h_next, 1 - kh)
            n_mxu = [(SH - r) // 16 for r in RU[kh]]
            off = np.cumsum([0] + n_mxu).tolist()
            vpu = sorted(((u, b, t) for u in range(NQB) for t in range(NT)
                          for b in range((RS[kh] - RU[kh][u]) // 16, RS[kh] // 16)),
                         key=lambda p: (p[0], p[1] // trun[kh], p[2], p[1]))
            ng = RS[1 - kh] // 8
            copies = [(d, range(g, min(g + kbg, ng))) for d in range(DH) for g in range(0, ng, kbg)]
            v0, v1 = vspan[kh]
            events = sorted([((a + 0.5) / off[-1], 0, a) for a in range(off[-1])]
                            + [(v0 + (v1 - v0) * (i + 0.5) / len(vpu), 1, i) for i in range(len(vpu))]
                            + [(kspan * (i + 0.5) / len(copies), 2, i) for i in range(len(copies))])

            def add_l(u, t, p):
                for g in (p[:8], p[8:]):
                    l[u][t] = g if l[u][t] is None else l[u][t] + g

            def mxu_piece(s, u, a):
                p = jnp.exp2(s)
                for t in range(NT):
                    add_l(u, t, p[:, t * 128:(t + 1) * 128])
                p_wr[pl.ds(u * PR + a * 8, 8), :] = _pack(p)

            def vpu_piece(u, b, t):
                s = [None, None]
                for d in range(DH):
                    kb = [pltpu.bitcast(p_rd[kb_slot(d, 2 * b + g)], F32) for g in range(2)]
                    qd = jnp.broadcast_to(qt_s[h, u, pl.ds(d, 1), pl.ds(t * 128, 128)], (8, 128))
                    for g in range(2):
                        s[g] = kb[g] * qd if d == 0 else s[g] + kb[g] * qd
                p = jnp.exp2(jnp.concatenate(s, axis=0))
                add_l(u, t, p)
                p_paced[pl.ds(u * PR + (SH - RS[kh]) // 2 + b * 8, 8), pl.ds(t * 128, 128)] = _pack(p)

            for period in range(NP):
                u, j = divmod(period, NKH)
                if period in ffn_at[kh]:
                    ffn_step(*ffn_at[kh][period])
                a0, a1 = n_mxu[u] * j // NKH, n_mxu[u] * (j + 1) // NKH
                k = _unpack(kh_bufs[kh][pl.ds(a0 * 8, (a1 - a0) * 8), :])
                s = jnp.dot(k[:, :DH], _unpack(qp_s[h, u]), preferred_element_type=F32)
                while events and (events[0][1] or events[0][2] < off[u] + a1):
                    _, kind, i = events.pop(0)
                    if kind == 0:
                        a = i - off[u]
                        mxu_piece(s[(a - a0) * 16:(a - a0 + 1) * 16], u, a)
                    elif kind == 1:
                        vpu_piece(*vpu[i])
                    else:
                        kb_prep(p_paced, h_next, 1 - kh, *copies[i])
                if period >= kh * plag:
                    pv_step(*divmod(period - kh * plag, NKH))
            for period in range(NP - kh * plag, NP):
                pv_step(*divmod(period, NKH))

        def head(h, carry):
            l_min, l_max = carry
            h_prev, h_next = jnp.maximum(h - 1, 0), jnp.minimum(h + 1, H - 1)
            zero = (h // H) * 16
            rows = pl.ds(pl.multiple_of(h * FR, FR), FR)
            inv, live = [], {}
            for u in range(NQB):
                r, l_min, l_max = inv_sum(u, l_min, l_max)
                inv.append(r)

            def pv_prev(u, j):
                live["o"] = (oc_s[u] if j == 0 else live["o"]) + pv_dot(h_prev, 1, pb_s, u, j)
                if j == NKH - 1:
                    ot_s[h_prev, u] = _pack(live["o"] * inv[u])

            def pv_this(u, j):
                pv = pv_dot(h, 0, pa_s, u, j)
                live["o"] = pv if j == 0 else live["o"] + pv
                if j == NKH - 1:
                    oc_s[u] = live["o"]

            def ffn_up(c, r):
                xn = _unpack(xn_s[pl.ds(pl.multiple_of(h * (FR // 2) + r // 2, 8), G1M // 2), :])
                hid = jnp.dot(xn, _unpack(w1_s[c]), preferred_element_type=F32)
                hid = hid + jnp.concatenate([b1_s[c]] * (G1M // 8), axis=0)
                act_s[pl.ds(r // 2, G1M // 2), pl.ds(c * 128, 128)] = _pack(_mish(hid))

            def ffn_down(n, c):
                kt, nt = (2, 2) if c == 12 else (4, 1)
                y = jnp.dot(_unpack(act_s[:, pl.ds(c * 128, kt * 128)]),
                            _unpack(w2_s[pl.ds(c * 64, kt * 64), pl.ds(n * 128, nt * 128)]),
                            preferred_element_type=F32)
                if c == 12:
                    acc_s[rows, pl.ds(n * 128, 128)] = live["y"] + y[:, :128]
                    live["y"] = y[:, 128:]
                else:
                    live["y"] = y if (c == 0 and n % 2 == 0) else live["y"] + y
                    if c == 8 and n % 2 == 1:
                        acc_s[rows, pl.ds(n * 128, 128)] = live["y"]

            l = [[None] * NT for _ in range(NQB)]
            score_step(h, 0, l, pa_s, pb_s, h, zero, pv_prev, ffn_up)
            score_step(h, 1, l, pb_s, pa_s, h_next, zero, pv_this, ffn_down)
            for u in range(NQB):
                l_s[u] = jnp.concatenate(l[u], axis=1)
            return l_min, l_max

        one = jnp.ones((1, TQ), F32)
        l_min, l_max = lax.fori_loop(0, H, head, (one, one))
        inv = []
        for u in range(NQB):
            r, l_min, l_max = inv_sum(u, l_min, l_max)
            inv.append(r)

        unsafe = jnp.min(jnp.where((l_min >= L_LO) & (l_max <= L_HI), 1.0, 0.0)) < 0.5

        @pl.when(unsafe)
        def _():
            def shifted_softmax(i, carry):
                h, u = i // NQB, i % NQB
                slot = lax.broadcasted_iota(jnp.int32, (64, TQ), 0) // 8
                q = _unpack(jnp.where(slot == h % 8, jnp.concatenate([qp_s[h, u]] * 8, axis=0), jnp.uint32(0)))

                def scores(j):
                    k = _unpack(k_s[h // 8, pl.ds(pl.multiple_of(j * (TK // 2), TK // 2), TK // 2), :])
                    return jnp.dot(k, q, preferred_element_type=F32)

                def row_max(j, m):
                    return jnp.maximum(m, jnp.max(scores(j), axis=0, keepdims=True))

                m = lax.fori_loop(0, S // TK, row_max, jnp.full((1, TQ), -jnp.inf, F32))

                def accumulate(j, c):
                    p = jnp.exp2(scores(j) - m)
                    return (c[0] + jnp.sum(p, axis=0, keepdims=True),
                            c[1] + jnp.dot(_unpack(vt_s[h, j]), p.astype(BF16), preferred_element_type=F32))

                l, o = lax.fori_loop(0, S // TK, accumulate, (jnp.zeros((1, TQ), F32), jnp.zeros((DH, TQ), F32)))
                ot_s[h, u] = _pack(o / l)
                return carry

            lax.fori_loop(0, H * NQB, shifted_softmax, 0)

        todo, o_last, out_cps = [(u, j) for u in range(NQB) for j in range(NKH)], {}, []

        def pv_last():
            u, j = todo.pop(0)
            o_last[u] = (oc_s[u] if j == 0 else o_last[u]) + pv_dot(H - 1, 1, pb_s, u, j)
            if j == NKH - 1:
                ot_s[H - 1, u] = jnp.where(unsafe, ot_s[H - 1, u], _pack(o_last[u] * inv[u]))

        for _ in range(NKH):
            pv_last()
        for i, r0 in enumerate(range(0, RB if LO else S, RB)):
            u, rows = r0 // TQ, pl.ds(r0, RB)
            y = x_v[rows, :].astype(F32) + acc_s[rows, :]
            for c in range(D // 128):
                assert not todo or todo[0][0] > u
                ot = jnp.concatenate([ot_s[h, u, :, pl.ds(r0 % TQ, RB)] for h in range(8 * c, 8 * c + 8)], axis=0)
                y = y + lax.dot_general(_unpack(ot), wo_v[pl.ds(c * 128, 128), :], (((0,), (0,)), ((), ())),
                                        preferred_element_type=F32)
                if todo:
                    pv_last()
            out_v[rows, :] = y.astype(out_v.dtype)
            out_cps.append(pltpu.make_async_copy(out_v.at[rows, :], out_hbm.at[0, rows, :], sems.at[i]))
            out_cps[-1].start()
        for c in out_cps:
            c.wait()

    def call(A_x, A_wqkv, A_wo, B_x, B_w1, B_b1, B_w2):
        del B_x
        _, S, D = A_x.shape
        F = B_w1.shape[1]
        NF = F // 128
        assert A_x.shape == (1, 2048, H * DH) and NF == 14
        vm = pltpu.VMEM
        hbm = pl.BlockSpec(memory_space=pl.ANY)
        p_shape = vm((S + NGM * 32, TQ), U32)
        return pl.pallas_call(
            kernel,
            out_shape=jax.ShapeDtypeStruct(A_x.shape, A_x.dtype),
            in_specs=[hbm] * 6,
            out_specs=hbm,
            scratch_shapes=[
                vm((S, D), BF16),
                vm((D, 3 * D), BF16),
                vm((D, D), BF16),
                vm((D, F), BF16),
                vm((F, D), BF16),
                vm((NF, D // 2, 128), U32),
                vm((F // 2, D), U32),
                vm((16, 8, 128), F32),
                vm((S // 2, D), U32),
                vm((D // 128, S // 2, 128), U32),
                vm((D // 128, 2, -(-NGM // 8) * 64, 128), F32),
                vm((H, S // TQ, DH, TQ), F32),
                vm((H, S // TK, 8, TK), U32),
                vm((H, S // TQ, 8, TQ), U32),
                vm((S // 4, 128), U32),
                vm((S // 4, 128), U32),
                vm((S // H // 2, 2048), U32),
                vm((S // TQ, DH, TQ), F32),
                vm((S // TQ, 8, TQ), F32),
                p_shape, p_shape,
                vm((H, S // TQ, 8, TQ), U32),
                vm((S, D), F32),
                vm((S, D), BF16),
                vm((NF, 128), BF16),
                pltpu.SemaphoreType.DMA((16,)),
            ],
            compiler_params=pltpu.CompilerParams(vmem_limit_bytes=100 << 20),
            name=name,
        )(A_x, A_wqkv, A_wo, B_w1, B_b1.reshape(NF, 128), B_w2)

    return call


@jax.jit
def pallas_parallel_sum__mha_block__dense_activation_mish__prompt_kernel(
    A_x: jax.Array,
    A_wqkv: jax.Array,
    A_wo: jax.Array,
    B_x: jax.Array,
    B_w1: jax.Array,
    B_b1: jax.Array,
    B_w2: jax.Array,
):
    return make()(A_x, A_wqkv, A_wo, B_x, B_w1, B_b1, B_w2)
```

```python
import jax
import jax.numpy as jnp
import numpy as np
from jax import lax
from jax.experimental import pallas as pl
from jax.experimental.pallas import tpu as pltpu

F32, BF16, U32 = jnp.float32, jnp.bfloat16, jnp.uint32
LOG2E = float(np.log2(np.e))
H, DH = 32, 16
TQ = 512
TK = 128
NT = TQ // 128
L_LO, L_HI = 2.0 ** -40, 2.0 ** 40

RS = (176, 192)
NGM = max(RS) // 8
V_SPAN = ((0, 1), (0.015, 1.03))
V_RUN = (5, 6)
K_SPAN, K_BATCH = 0.97, 6
CUT = (3, 4)
FFN_START = (1, 0)
PV_LAG = 1
FM = 32
X0, R1, RB = 768, 128, 256

_reciprocal = getattr(pltpu, "reciprocal", None) or pl.reciprocal


def _pack(x):
    return pltpu.bitcast(x.astype(BF16), U32)


def _unpack(x):
    return pltpu.bitcast(x, BF16)


def _mish(h2):
    e = jnp.exp2(jnp.minimum(h2, 30.0))
    n = e * (e + 2.0)
    return h2 * (n * _reciprocal(n + 2.0, approx=True))


def _kernel(x_hbm, wqkv_hbm, wo_hbm, w1_hbm, b1_hbm, w2_hbm, out_hbm,
           x_v, wqkv_v, wo_v, w1_v, w2_v, w1_s, w2_s, b1_s, xn_s, k_s, kf_s, qt_s, vt_s, qp_s,
           kha_s, khb_s, act_s, oc_s, l_s, pa_s, pb_s, ot_s, acc_s, out_v, b1_v, sems):
    S, D = x_v.shape
    NF = w1_v.shape[1] // 128
    NQB = S // TQ
    SH = S // 2
    NKH = SH // TK
    NP = NQB * NKH
    PR = SH // 2
    FR = S // H
    kh_bufs = (kha_s, khb_s)

    def x_cp(r0, r1, sem):
        return pltpu.make_async_copy(x_hbm.at[0, pl.ds(r0, r1 - r0), :], x_v.at[pl.ds(r0, r1 - r0), :], sems.at[sem])

    def wqkv_cp(i):
        return pltpu.make_async_copy(wqkv_hbm.at[:, pl.ds(i * D, D)], wqkv_v.at[:, pl.ds(i * D, D)], sems.at[2 + i])

    late_cps = [pltpu.make_async_copy(src, dst, sems.at[5 + i])
                for i, (src, dst) in enumerate(((w1_hbm, w1_v), (w2_hbm, w2_v), (wo_hbm, wo_v), (b1_hbm, b1_v)))]

    def kb_slot(d, g):
        i = g * DH + d
        return pl.ds(NQB * PR + (i // NT) * 8, 8), pl.ds((i % NT) * 128, 128)

    def kb_prep(dst, h, kh, d, groups):
        idx = jnp.full((8, 128), ((h % 8) * DH + d) & 127, U32)
        for g in groups:
            kb = jnp.take_along_axis(kf_s[h // 8, kh, pl.ds(g * 8, 8), :], idx, axis=1)
            dst[kb_slot(d, g)] = pltpu.bitcast(kb, U32)

    def kh_prep(h, kh):
        n = (SH - RS[kh]) // 2
        idx = (lax.broadcasted_iota(jnp.int32, (8, 128), 1) % DH + (h % 8) * DH).astype(U32)
        for r in range(0, n, 8):
            k = k_s[h // 8, pl.ds(kh * SH // 2 + r, 8), :]
            kh_bufs[kh][pl.ds(r, 8), :] = jnp.take_along_axis(k, idx, axis=1)

    def pv_dot(h, kh, p_ref, u, j):
        p = _unpack(p_ref[pl.ds(u * PR + j * TK // 2, TK // 2), :])
        return jnp.dot(_unpack(vt_s[h, kh * NKH + j]), p, preferred_element_type=F32)

    def inv_sum(u, l_min, l_max):
        l = jnp.sum(l_s[u], axis=0, keepdims=True)
        r = _reciprocal(l, approx=True)
        return r * (2.0 - l * r), jnp.minimum(l_min, l), jnp.maximum(l_max, l)

    def layernorm(r0, n):
        x = x_v[pl.ds(r0, n), :].astype(F32)
        xc = x - jnp.mean(x, axis=-1, keepdims=True)
        var = jnp.mean(xc * xc, axis=-1, keepdims=True)
        xn_s[pl.ds(r0 // 2, n // 2), :] = _pack(xc * (lax.rsqrt(var + 1e-5) * LOG2E))

    def project(r0, n, i):
        return jnp.dot(_unpack(xn_s[pl.ds(r0 // 2, n // 2), :]), wqkv_v[:, pl.ds(i * D, D)],
                       preferred_element_type=F32)

    def k_proj(r0, n):
        k = project(r0, n, 1)
        kp = _pack(k)
        kh = r0 // SH
        v0 = (kh + 1) * SH - RS[kh]
        lo = max(r0, v0)
        for c in range(D // 128):
            k_s[c, pl.ds(r0 // 2, n // 2), :] = kp[:, c * 128:(c + 1) * 128]
            if lo < r0 + n:
                kf_s[c, kh, pl.ds(lo - v0, r0 + n - lo), :] = k[lo - r0:, c * 128:(c + 1) * 128]

    def qv_proj(r0):
        q = (project(r0, RB, 0) * (DH ** -0.5 / LOG2E)).T
        v = project(r0, RB, 2).T
        u, cols = r0 // TQ, pl.ds(r0 % TQ, RB)
        for h in range(H):
            qt_s[h, u, :, cols] = q[h * DH:(h + 1) * DH]
            qp_s[h, u, :, cols] = _pack(q[h * DH:(h + 1) * DH])
            for t in range(RB // TK):
                vt_s[h, r0 // TK + t] = _pack(v[h * DH:(h + 1) * DH, t * TK:(t + 1) * TK])

    x_cp(0, X0, 0).start()
    wqkv_cp(1).start()
    pb_s[pl.ds(0, NQB * PR), :] = jnp.zeros((NQB * PR, TQ), U32)
    oc_s[...] = jnp.zeros(oc_s.shape, F32)
    ot_s[H - 1] = jnp.zeros(ot_s.shape[1:], U32)
    l_s[...] = jnp.full(l_s.shape, 0.125, F32)
    wqkv_cp(0).start()
    x_cp(0, X0, 0).wait()
    wqkv_cp(1).wait()
    wqkv_cp(2).start()
    for r0 in range(0, X0, R1):
        layernorm(r0, R1)
        if r0 == X0 // 2 // R1 * R1:
            x_cp(X0, S, 1).start()
        k_proj(r0, R1)
    wqkv_cp(0).wait()
    wqkv_cp(2).wait()
    for r0 in range(0, X0 - RB, RB):
        qv_proj(r0)
    x_cp(X0, S, 1).wait()
    for c in late_cps:
        c.start()
    qv_proj(X0 - RB)
    for r0 in range(X0, S, RB):
        layernorm(r0, RB)
        if r0 + RB < S:
            k_proj(r0, RB)
    kh_prep(0, 0)
    for d in range(DH):
        kb_prep(pb_s, 0, 0, d, range(RS[0] // 8))
    for r0 in range(X0, S - RB, RB):
        qv_proj(r0)
    for c in late_cps:
        c.wait()
    qv_proj(S - RB)
    k_proj(S - RB, RB)
    for c in range(NF):
        w1_s[c] = pltpu.bitcast(w1_v[:, pl.ds(c * 128, 128)], U32)
    w2_s[...] = pltpu.bitcast(w2_v[...], U32)
    b1 = b1_v[...].astype(F32) * LOG2E
    for c in range(NF):
        b1_s[c] = jnp.broadcast_to(b1[c:c + 1, :], (8, 128))

    ffn_ops = ([(c, r) for r in range(0, FR, FM) for c in range(NF)],
               [op + (r,) for r in range(0, FR, FM) for n in (0, 2)
                for op in ((n, 0), (n, 4), (n, 8), (n, 12), (n + 1, 0), (n + 1, 4), (n + 1, 8))])
    ffn_at = [{lo + i * (NP - lo) // len(ops): op for i, op in enumerate(ops)} for ops, lo in zip(ffn_ops, FFN_START)]
    assert [len(a) for a in ffn_at] == [len(ops) for ops in ffn_ops]

    def score_step(h, kh, l, p_wr, p_rd, h_next, zero, pv_step, ffn_step):
        p_paced = p_wr.at[pl.ds(pl.multiple_of(zero, 16), p_wr.shape[0])]
        kh_prep(h_next, 1 - kh)
        n_mxu = (SH - RS[kh]) // 16
        vpu = sorted(((u, b, t) for u in range(NQB) for t in range(NT) for b in range(RS[kh] // 16)),
                     key=lambda p: (p[0], p[1] // V_RUN[kh], p[2], p[1]))
        ng = RS[1 - kh] // 8
        copies = [(d, range(g, min(g + K_BATCH, ng))) for d in range(DH) for g in range(0, ng, K_BATCH)]
        v0, v1 = V_SPAN[kh]
        events = sorted([((a + 0.5) / (NQB * n_mxu), 0, a) for a in range(NQB * n_mxu)]
                        + [(v0 + (v1 - v0) * (i + 0.5) / len(vpu), 1, i) for i in range(len(vpu))]
                        + [(K_SPAN * (i + 0.5) / len(copies), 2, i) for i in range(len(copies))])

        def add_l(u, t, p):
            for g in (p[:8], p[8:]):
                l[u][t] = g if l[u][t] is None else l[u][t] + g

        def mxu_piece(s, u, a):
            p = jnp.exp2(s)
            for t in range(NT):
                add_l(u, t, p[:, t * 128:(t + 1) * 128])
            p_wr[pl.ds(u * PR + a * 8, 8), :] = _pack(p)

        def vpu_piece(u, b, t):
            s = [None, None]
            for d in range(DH):
                kb = [pltpu.bitcast(p_rd[kb_slot(d, 2 * b + g)], F32) for g in range(2)]
                qd = jnp.broadcast_to(qt_s[h, u, pl.ds(d, 1), pl.ds(t * 128, 128)], (8, 128))
                for g in range(2):
                    s[g] = kb[g] * qd if d == 0 else s[g] + kb[g] * qd
            p = jnp.exp2(jnp.concatenate(s, axis=0))
            add_l(u, t, p)
            p_paced[pl.ds(u * PR + (n_mxu + b) * 8, 8), pl.ds(t * 128, 128)] = _pack(p)

        for period in range(NP):
            u, j = divmod(period, NKH)
            lo, hi = n_mxu * j // NKH, n_mxu * (j + 1) // NKH
            mid = min(lo + CUT[kh], hi) if period in ffn_at[kh] else lo
            for part, (a0, a1) in enumerate(((lo, mid), (mid, hi))):
                if part == 1 and period in ffn_at[kh]:
                    ffn_step(*ffn_at[kh][period])
                if a0 == a1:
                    continue
                k = _unpack(kh_bufs[kh][pl.ds(a0 * 8, (a1 - a0) * 8), :])
                s = jnp.dot(k[:, :DH], _unpack(qp_s[h, u]), preferred_element_type=F32)
                while events and (events[0][1] or events[0][2] < u * n_mxu + a1):
                    _, kind, i = events.pop(0)
                    if kind == 0:
                        a = i - u * n_mxu
                        mxu_piece(s[(a - a0) * 16:(a - a0 + 1) * 16], u, a)
                    elif kind == 1:
                        vpu_piece(*vpu[i])
                    else:
                        kb_prep(p_paced, h_next, 1 - kh, *copies[i])
            if period >= kh * PV_LAG:
                pv_step(*divmod(period - kh * PV_LAG, NKH))
        for period in range(NP - kh * PV_LAG, NP):
            pv_step(*divmod(period, NKH))

    def head(h, carry):
        l_min, l_max = carry
        h_prev, h_next = jnp.maximum(h - 1, 0), jnp.minimum(h + 1, H - 1)
        zero = (h // H) * 16
        inv, live = [], {}
        for u in range(NQB):
            r, l_min, l_max = inv_sum(u, l_min, l_max)
            inv.append(r)

        def pv_prev(u, j):
            live["o"] = (oc_s[u] if j == 0 else live["o"]) + pv_dot(h_prev, 1, pb_s, u, j)
            if j == NKH - 1:
                ot_s[h_prev, u] = _pack(live["o"] * inv[u])

        def pv_this(u, j):
            pv = pv_dot(h, 0, pa_s, u, j)
            live["o"] = pv if j == 0 else live["o"] + pv
            if j == NKH - 1:
                oc_s[u] = live["o"]

        def ffn_up(c, r):
            xn = _unpack(xn_s[pl.ds(pl.multiple_of(h * (FR // 2) + r // 2, 8), FM // 2), :])
            hid = jnp.dot(xn, _unpack(w1_s[c]), preferred_element_type=F32)
            hid = hid + jnp.concatenate([b1_s[c]] * (FM // 8), axis=0)
            act_s[pl.ds(r // 2, FM // 2), pl.ds(c * 128, 128)] = _pack(_mish(hid))

        def ffn_down(n, c, r):
            rows = pl.ds(pl.multiple_of(h * FR + r, FM), FM)
            kt, nt = (2, 2) if c == 12 else (4, 1)
            y = jnp.dot(_unpack(act_s[pl.ds(r // 2, FM // 2), pl.ds(c * 128, kt * 128)]),
                        _unpack(w2_s[pl.ds(c * 64, kt * 64), pl.ds(n * 128, nt * 128)]),
                        preferred_element_type=F32)
            if c == 12:
                acc_s[rows, pl.ds(n * 128, 128)] = live["y"] + y[:, :128]
                live["y"] = y[:, 128:]
            else:
                live["y"] = y if (c == 0 and n % 2 == 0) else live["y"] + y
                if c == 8 and n % 2 == 1:
                    acc_s[rows, pl.ds(n * 128, 128)] = live["y"]

        l = [[None] * NT for _ in range(NQB)]
        score_step(h, 0, l, pa_s, pb_s, h, zero, pv_prev, ffn_up)
        score_step(h, 1, l, pb_s, pa_s, h_next, zero, pv_this, ffn_down)
        for u in range(NQB):
            l_s[u] = jnp.concatenate(l[u], axis=1)
        return l_min, l_max

    one = jnp.ones((1, TQ), F32)
    l_min, l_max = lax.fori_loop(0, H, head, (one, one))
    inv = []
    for u in range(NQB):
        r, l_min, l_max = inv_sum(u, l_min, l_max)
        inv.append(r)

    unsafe = jnp.min(jnp.where((l_min >= L_LO) & (l_max <= L_HI), 1.0, 0.0)) < 0.5

    @pl.when(unsafe)
    def _():
        def shifted_softmax(i, carry):
            h, u = i // NQB, i % NQB
            slot = lax.broadcasted_iota(jnp.int32, (64, TQ), 0) // 8
            q = _unpack(jnp.where(slot == h % 8, jnp.concatenate([qp_s[h, u]] * 8, axis=0), jnp.uint32(0)))

            def scores(j):
                k = _unpack(k_s[h // 8, pl.ds(pl.multiple_of(j * (TK // 2), TK // 2), TK // 2), :])
                return jnp.dot(k, q, preferred_element_type=F32)

            def row_max(j, m):
                return jnp.maximum(m, jnp.max(scores(j), axis=0, keepdims=True))

            m = lax.fori_loop(0, S // TK, row_max, jnp.full((1, TQ), -jnp.inf, F32))

            def accumulate(j, c):
                p = jnp.exp2(scores(j) - m)
                return (c[0] + jnp.sum(p, axis=0, keepdims=True),
                        c[1] + jnp.dot(_unpack(vt_s[h, j]), p.astype(BF16), preferred_element_type=F32))

            l, o = lax.fori_loop(0, S // TK, accumulate, (jnp.zeros((1, TQ), F32), jnp.zeros((DH, TQ), F32)))
            ot_s[h, u] = _pack(o / l)
            return carry

        lax.fori_loop(0, H * NQB, shifted_softmax, 0)

    todo, o_last, out_cps = [(u, j) for u in range(NQB) for j in range(NKH)], {}, []

    def pv_last():
        u, j = todo.pop(0)
        o_last[u] = (oc_s[u] if j == 0 else o_last[u]) + pv_dot(H - 1, 1, pb_s, u, j)
        if j == NKH - 1:
            ot_s[H - 1, u] = jnp.where(unsafe, ot_s[H - 1, u], _pack(o_last[u] * inv[u]))

    for _ in range(NKH):
        pv_last()
    for i, r0 in enumerate(range(0, S, RB)):
        u, rows = r0 // TQ, pl.ds(r0, RB)
        y = acc_s[rows, :]
        for c in range(D // 128):
            assert not todo or todo[0][0] > u
            ot = jnp.concatenate([ot_s[h, u, :, pl.ds(r0 % TQ, RB)] for h in range(8 * c, 8 * c + 8)], axis=0)
            y = y + lax.dot_general(_unpack(ot), wo_v[pl.ds(c * 128, 128), :], (((0,), (0,)), ((), ())),
                                    preferred_element_type=F32)
            if todo:
                pv_last()
        out_v[rows, :] = (x_v[rows, :].astype(F32) + y * (1.0 / LOG2E)).astype(out_v.dtype)
        out_cps.append(pltpu.make_async_copy(out_v.at[rows, :], out_hbm.at[0, rows, :], sems.at[i]))
        out_cps[-1].start()
    for c in out_cps:
        c.wait()


@jax.jit
def pallas_parallel_sum__mha_block__dense_activation_mish__prompt_kernel(
    A_x: jax.Array,
    A_wqkv: jax.Array,
    A_wo: jax.Array,
    B_x: jax.Array,
    B_w1: jax.Array,
    B_b1: jax.Array,
    B_w2: jax.Array,
):
    del B_x
    _, S, D = A_x.shape
    F = B_w1.shape[1]
    NF = F // 128
    assert A_x.shape == (1, 2048, H * DH) and NF == 14
    vm = pltpu.VMEM
    hbm = pl.BlockSpec(memory_space=pl.ANY)
    p_shape = vm((S + NGM * 32, TQ), U32)
    return pl.pallas_call(
        _kernel,
        out_shape=jax.ShapeDtypeStruct(A_x.shape, A_x.dtype),
        in_specs=[hbm] * 6,
        out_specs=hbm,
        scratch_shapes=[
            vm((S, D), BF16),
            vm((D, 3 * D), BF16),
            vm((D, D), BF16),
            vm((D, F), BF16),
            vm((F, D), BF16),
            vm((NF, D // 2, 128), U32),
            vm((F // 2, D), U32),
            vm((16, 8, 128), F32),
            vm((S // 2, D), U32),
            vm((D // 128, S // 2, 128), U32),
            vm((D // 128, 2, -(-NGM // 8) * 64, 128), F32),
            vm((H, S // TQ, DH, TQ), F32),
            vm((H, S // TK, 8, TK), U32),
            vm((H, S // TQ, 8, TQ), U32),
            vm((S // 4, 128), U32),
            vm((S // 4, 128), U32),
            vm((S // H // 2, 2048), U32),
            vm((S // TQ, DH, TQ), F32),
            vm((S // TQ, 8, TQ), F32),
            p_shape, p_shape,
            vm((H, S // TQ, 8, TQ), U32),
            vm((S, D), F32),
            vm((S, D), BF16),
            vm((NF, 128), BF16),
            pltpu.SemaphoreType.DMA((16,)),
        ],
        compiler_params=pltpu.CompilerParams(vmem_limit_bytes=100 << 20),
    )(A_x, A_wqkv, A_wo, B_w1, B_b1.reshape(NF, 128), B_w2)
```

```python
import jax
import jax.numpy as jnp
import numpy as np
from jax import lax
from jax.experimental import pallas as pl
from jax.experimental.pallas import tpu as pltpu

F32, BF16, U32 = jnp.float32, jnp.bfloat16, jnp.uint32
LOG2E = float(np.log2(np.e))
H, DH = 32, 16
TQ = 512
TK = 128
NT = TQ // 128
L_LO, L_HI = 2.0 ** -40, 2.0 ** 40

RS = (176, 192)
NGM = max(RS) // 8
V_SPAN = ((0, 1), (0.015, 1.03))
V_RUN = (5, 6)
K_SPAN, K_BATCH = 0.97, 6
CUT = (3, 4)
FFN_START = (1, 0)
PV_LAG = 1
FM = 32
XA, X0 = 256, 768
R1, RB, OL = 128, 256, 128

_reciprocal = getattr(pltpu, "reciprocal", None) or pl.reciprocal


def _pack(x):
    return pltpu.bitcast(x.astype(BF16), U32)


def _unpack(x):
    return pltpu.bitcast(x, BF16)


def _mish(h2):
    e = jnp.exp2(jnp.minimum(h2, 30.0))
    n = e * (e + 2.0)
    return h2 * (n * _reciprocal(n + 2.0, approx=True))


def _kernel(x_hbm, wqkv_hbm, wo_hbm, w1_hbm, b1_hbm, w2_hbm, out_hbm,
           x_v, wqkv_v, wo_v, w1_v, w2_v, w1_s, w2_s, b1_s, xn_s, k_s, kf_s, qt_s, vt_s, qp_s,
           kha_s, khb_s, act_s, oc_s, l_s, pa_s, pb_s, ot_s, acc_s, out_v, b1_v, sems):
    S, D = x_v.shape
    NF = w1_v.shape[1] // 128
    NQB = S // TQ
    SH = S // 2
    NKH = SH // TK
    NP = NQB * NKH
    PR = SH // 2
    FR = S // H
    kh_bufs = (kha_s, khb_s)

    def x_cp(r0, r1, sem):
        return pltpu.make_async_copy(x_hbm.at[0, pl.ds(r0, r1 - r0), :], x_v.at[pl.ds(r0, r1 - r0), :], sems.at[sem])

    def wqkv_cp(i):
        return pltpu.make_async_copy(wqkv_hbm.at[:, pl.ds(i * D, D)], wqkv_v.at[:, pl.ds(i * D, D)], sems.at[2 + i])

    late_cps = [pltpu.make_async_copy(src, dst, sems.at[5 + i])
                for i, (src, dst) in enumerate(((w1_hbm, w1_v), (w2_hbm, w2_v), (wo_hbm, wo_v), (b1_hbm, b1_v)))]

    def kb_slot(d, g):
        i = g * DH + d
        return pl.ds(NQB * PR + (i // NT) * 8, 8), pl.ds((i % NT) * 128, 128)

    def kb_prep(dst, h, kh, d, groups):
        idx = jnp.full((8, 128), ((h % 8) * DH + d) & 127, U32)
        for g in groups:
            kb = jnp.take_along_axis(kf_s[h // 8, kh, pl.ds(g * 8, 8), :], idx, axis=1)
            dst[kb_slot(d, g)] = pltpu.bitcast(kb, U32)

    def kh_prep(h, kh):
        n = (SH - RS[kh]) // 2
        idx = (lax.broadcasted_iota(jnp.int32, (8, 128), 1) % DH + (h % 8) * DH).astype(U32)
        for r in range(0, n, 8):
            k = k_s[h // 8, pl.ds(kh * SH // 2 + r, 8), :]
            kh_bufs[kh][pl.ds(r, 8), :] = jnp.take_along_axis(k, idx, axis=1)

    def pv_dot(h, kh, p_ref, u, j):
        p = _unpack(p_ref[pl.ds(u * PR + j * TK // 2, TK // 2), :])
        return jnp.dot(_unpack(vt_s[h, kh * NKH + j]), p, preferred_element_type=F32)

    def inv_sum(u, l_min, l_max):
        l = jnp.sum(l_s[u], axis=0, keepdims=True)
        r = _reciprocal(l, approx=True)
        return r * (2.0 - l * r), jnp.minimum(l_min, l), jnp.maximum(l_max, l)

    def layernorm(r0, n):
        x = x_v[pl.ds(r0, n), :].astype(F32)
        xc = x - jnp.mean(x, axis=-1, keepdims=True)
        var = jnp.mean(xc * xc, axis=-1, keepdims=True)
        xn_s[pl.ds(r0 // 2, n // 2), :] = _pack(xc * (lax.rsqrt(var + 1e-5) * LOG2E))

    def project(r0, n, i):
        return jnp.dot(_unpack(xn_s[pl.ds(r0 // 2, n // 2), :]), wqkv_v[:, pl.ds(i * D, D)],
                       preferred_element_type=F32)

    def k_proj(r0, n):
        k = project(r0, n, 1)
        kp = _pack(k)
        kh = r0 // SH
        v0 = (kh + 1) * SH - RS[kh]
        lo = max(r0, v0)
        for c in range(D // 128):
            k_s[c, pl.ds(r0 // 2, n // 2), :] = kp[:, c * 128:(c + 1) * 128]
            if lo < r0 + n:
                kf_s[c, kh, pl.ds(lo - v0, r0 + n - lo), :] = k[lo - r0:, c * 128:(c + 1) * 128]

    def qv_proj(r0):
        q = (project(r0, RB, 0) * (DH ** -0.5 / LOG2E)).T
        v = project(r0, RB, 2).T
        u, cols = r0 // TQ, pl.ds(r0 % TQ, RB)
        for h in range(H):
            qt_s[h, u, :, cols] = q[h * DH:(h + 1) * DH]
            qp_s[h, u, :, cols] = _pack(q[h * DH:(h + 1) * DH])
            for t in range(RB // TK):
                vt_s[h, r0 // TK + t] = _pack(v[h * DH:(h + 1) * DH, t * TK:(t + 1) * TK])

    x_cp(0, XA, 0).start()
    wqkv_cp(1).start()
    pb_s[pl.ds(0, NQB * PR), :] = jnp.zeros((NQB * PR, TQ), U32)
    oc_s[...] = jnp.zeros(oc_s.shape, F32)
    ot_s[H - 1] = jnp.zeros(ot_s.shape[1:], U32)
    l_s[...] = jnp.full(l_s.shape, 0.125, F32)
    x_cp(XA, X0, 9).start()
    x_cp(0, XA, 0).wait()
    wqkv_cp(1).wait()
    wqkv_cp(0).start()
    wqkv_cp(2).start()
    for r0 in range(0, XA, R1):
        layernorm(r0, R1)
        if r0 + R1 < XA:
            k_proj(r0, R1)
    x_cp(XA, X0, 9).wait()
    k_proj(XA - R1, R1)
    for r0 in range(XA, X0, R1):
        layernorm(r0, R1)
        if r0 == X0 - 2 * R1:
            x_cp(X0, S, 1).start()
        k_proj(r0, R1)
    wqkv_cp(0).wait()
    wqkv_cp(2).wait()
    for r0 in range(0, X0 - RB, RB):
        qv_proj(r0)
    x_cp(X0, S, 1).wait()
    for c in late_cps:
        c.start()
    qv_proj(X0 - RB)
    for r0 in range(X0, S, R1):
        layernorm(r0, R1)
        if r0 + RB < S:
            k_proj(r0, R1)
    kh_prep(0, 0)
    for d in range(DH):
        kb_prep(pb_s, 0, 0, d, range(RS[0] // 8))
    for r0 in range(X0, S - RB, RB):
        qv_proj(r0)
    for c in late_cps:
        c.wait()
    qv_proj(S - RB)
    k_proj(S - RB, RB)
    for c in range(NF):
        w1_s[c] = pltpu.bitcast(w1_v[:, pl.ds(c * 128, 128)], U32)
    w2_s[...] = pltpu.bitcast(w2_v[...], U32)
    b1 = b1_v[...].astype(F32) * LOG2E
    for c in range(NF):
        b1_s[c] = jnp.broadcast_to(b1[c:c + 1, :], (8, 128))

    ffn_ops = ([(c, r) for r in range(0, FR, FM) for c in range(NF)],
               [op + (r,) for r in range(0, FR, FM) for n in (0, 2)
                for op in ((n, 0), (n, 4), (n, 8), (n, 12), (n + 1, 0), (n + 1, 4), (n + 1, 8))])
    ffn_at = [{lo + i * (NP - lo) // len(ops): op for i, op in enumerate(ops)} for ops, lo in zip(ffn_ops, FFN_START)]
    assert [len(a) for a in ffn_at] == [len(ops) for ops in ffn_ops]

    def score_step(h, kh, l, p_wr, p_rd, h_next, zero, pv_step, ffn_step):
        p_paced = p_wr.at[pl.ds(pl.multiple_of(zero, 16), p_wr.shape[0])]
        kh_prep(h_next, 1 - kh)
        n_mxu = (SH - RS[kh]) // 16
        vpu = sorted(((u, b, t) for u in range(NQB) for t in range(NT) for b in range(RS[kh] // 16)),
                     key=lambda p: (p[0], p[1] // V_RUN[kh], p[2], p[1]))
        ng = RS[1 - kh] // 8
        copies = [(d, range(g, min(g + K_BATCH, ng))) for d in range(DH) for g in range(0, ng, K_BATCH)]
        v0, v1 = V_SPAN[kh]
        events = sorted([((a + 0.5) / (NQB * n_mxu), 0, a) for a in range(NQB * n_mxu)]
                        + [(v0 + (v1 - v0) * (i + 0.5) / len(vpu), 1, i) for i in range(len(vpu))]
                        + [(K_SPAN * (i + 0.5) / len(copies), 2, i) for i in range(len(copies))])

        def add_l(u, t, p):
            for g in (p[:8], p[8:]):
                l[u][t] = g if l[u][t] is None else l[u][t] + g

        def mxu_piece(s, u, a):
            p = jnp.exp2(s)
            for t in range(NT):
                add_l(u, t, p[:, t * 128:(t + 1) * 128])
            p_wr[pl.ds(u * PR + a * 8, 8), :] = _pack(p)

        def vpu_piece(u, b, t):
            s = [None, None]
            for d in range(DH):
                kb = [pltpu.bitcast(p_rd[kb_slot(d, 2 * b + g)], F32) for g in range(2)]
                qd = jnp.broadcast_to(qt_s[h, u, pl.ds(d, 1), pl.ds(t * 128, 128)], (8, 128))
                for g in range(2):
                    s[g] = kb[g] * qd if d == 0 else s[g] + kb[g] * qd
            p = jnp.exp2(jnp.concatenate(s, axis=0))
            add_l(u, t, p)
            p_paced[pl.ds(u * PR + (n_mxu + b) * 8, 8), pl.ds(t * 128, 128)] = _pack(p)

        for period in range(NP):
            u, j = divmod(period, NKH)
            lo, hi = n_mxu * j // NKH, n_mxu * (j + 1) // NKH
            mid = min(lo + CUT[kh], hi) if period in ffn_at[kh] else lo
            for part, (a0, a1) in enumerate(((lo, mid), (mid, hi))):
                if part == 1 and period in ffn_at[kh]:
                    ffn_step(*ffn_at[kh][period])
                if a0 == a1:
                    continue
                k = _unpack(kh_bufs[kh][pl.ds(a0 * 8, (a1 - a0) * 8), :])
                s = jnp.dot(k[:, :DH], _unpack(qp_s[h, u]), preferred_element_type=F32)
                while events and (events[0][1] or events[0][2] < u * n_mxu + a1):
                    _, kind, i = events.pop(0)
                    if kind == 0:
                        a = i - u * n_mxu
                        mxu_piece(s[(a - a0) * 16:(a - a0 + 1) * 16], u, a)
                    elif kind == 1:
                        vpu_piece(*vpu[i])
                    else:
                        kb_prep(p_paced, h_next, 1 - kh, *copies[i])
            if period >= kh * PV_LAG:
                pv_step(*divmod(period - kh * PV_LAG, NKH))
        for period in range(NP - kh * PV_LAG, NP):
            pv_step(*divmod(period, NKH))

    def head(h, carry):
        l_min, l_max = carry
        h_prev, h_next = jnp.maximum(h - 1, 0), jnp.minimum(h + 1, H - 1)
        zero = (h // H) * 16
        inv, live = [], {}
        for u in range(NQB):
            r, l_min, l_max = inv_sum(u, l_min, l_max)
            inv.append(r)

        def pv_prev(u, j):
            live["o"] = (oc_s[u] if j == 0 else live["o"]) + pv_dot(h_prev, 1, pb_s, u, j)
            if j == NKH - 1:
                ot_s[h_prev, u] = _pack(live["o"] * inv[u])

        def pv_this(u, j):
            pv = pv_dot(h, 0, pa_s, u, j)
            live["o"] = pv if j == 0 else live["o"] + pv
            if j == NKH - 1:
                oc_s[u] = live["o"]

        def ffn_up(c, r):
            xn = _unpack(xn_s[pl.ds(pl.multiple_of(h * (FR // 2) + r // 2, 8), FM // 2), :])
            hid = jnp.dot(xn, _unpack(w1_s[c]), preferred_element_type=F32)
            hid = hid + jnp.concatenate([b1_s[c]] * (FM // 8), axis=0)
            act_s[pl.ds(r // 2, FM // 2), pl.ds(c * 128, 128)] = _pack(_mish(hid))

        def ffn_down(n, c, r):
            rows = pl.ds(pl.multiple_of(h * FR + r, FM), FM)
            kt, nt = (2, 2) if c == 12 else (4, 1)
            y = jnp.dot(_unpack(act_s[pl.ds(r // 2, FM // 2), pl.ds(c * 128, kt * 128)]),
                        _unpack(w2_s[pl.ds(c * 64, kt * 64), pl.ds(n * 128, nt * 128)]),
                        preferred_element_type=F32)
            if c == 12:
                acc_s[rows, pl.ds(n * 128, 128)] = live["y"] + y[:, :128]
                live["y"] = y[:, 128:]
            else:
                live["y"] = y if (c == 0 and n % 2 == 0) else live["y"] + y
                if c == 8 and n % 2 == 1:
                    acc_s[rows, pl.ds(n * 128, 128)] = live["y"]

        l = [[None] * NT for _ in range(NQB)]
        score_step(h, 0, l, pa_s, pb_s, h, zero, pv_prev, ffn_up)
        score_step(h, 1, l, pb_s, pa_s, h_next, zero, pv_this, ffn_down)
        for u in range(NQB):
            l_s[u] = jnp.concatenate(l[u], axis=1)
        return l_min, l_max

    one = jnp.ones((1, TQ), F32)
    l_min, l_max = lax.fori_loop(0, H, head, (one, one))
    inv = []
    for u in range(NQB):
        r, l_min, l_max = inv_sum(u, l_min, l_max)
        inv.append(r)

    unsafe = jnp.min(jnp.where((l_min >= L_LO) & (l_max <= L_HI), 1.0, 0.0)) < 0.5

    @pl.when(unsafe)
    def _():
        def shifted_softmax(i, carry):
            h, u = i // NQB, i % NQB
            slot = lax.broadcasted_iota(jnp.int32, (64, TQ), 0) // 8
            q = _unpack(jnp.where(slot == h % 8, jnp.concatenate([qp_s[h, u]] * 8, axis=0), jnp.uint32(0)))

            def scores(j):
                k = _unpack(k_s[h // 8, pl.ds(pl.multiple_of(j * (TK // 2), TK // 2), TK // 2), :])
                return jnp.dot(k, q, preferred_element_type=F32)

            def row_max(j, m):
                return jnp.maximum(m, jnp.max(scores(j), axis=0, keepdims=True))

            m = lax.fori_loop(0, S // TK, row_max, jnp.full((1, TQ), -jnp.inf, F32))

            def accumulate(j, c):
                p = jnp.exp2(scores(j) - m)
                return (c[0] + jnp.sum(p, axis=0, keepdims=True),
                        c[1] + jnp.dot(_unpack(vt_s[h, j]), p.astype(BF16), preferred_element_type=F32))

            l, o = lax.fori_loop(0, S // TK, accumulate, (jnp.zeros((1, TQ), F32), jnp.zeros((DH, TQ), F32)))
            ot_s[h, u] = _pack(o / l)
            return carry

        lax.fori_loop(0, H * NQB, shifted_softmax, 0)

    todo, o_last, out_cps = [(u, j) for u in range(NQB) for j in range(NKH)], {}, []

    def pv_last():
        u, j = todo.pop(0)
        o_last[u] = (oc_s[u] if j == 0 else o_last[u]) + pv_dot(H - 1, 1, pb_s, u, j)
        if j == NKH - 1:
            ot_s[H - 1, u] = jnp.where(unsafe, ot_s[H - 1, u], _pack(o_last[u] * inv[u]))

    for _ in range(NKH):
        pv_last()
    for r0 in range(0, S, RB):
        u, rows = r0 // TQ, pl.ds(r0, RB)
        y = acc_s[rows, :]
        for c in range(D // 128):
            assert not todo or todo[0][0] > u
            ot = jnp.concatenate([ot_s[h, u, :, pl.ds(r0 % TQ, RB)] for h in range(8 * c, 8 * c + 8)], axis=0)
            y = y + lax.dot_general(_unpack(ot), wo_v[pl.ds(c * 128, 128), :], (((0,), (0,)), ((), ())),
                                    preferred_element_type=F32)
            if todo:
                pv_last()
        n = RB if r0 + RB < S else OL
        for r in range(0, RB, n):
            rows = pl.ds(r0 + r, n)
            out_v[rows, :] = (x_v[rows, :].astype(F32) + y[r:r + n] * (1.0 / LOG2E)).astype(out_v.dtype)
            out_cps.append(pltpu.make_async_copy(out_v.at[rows, :], out_hbm.at[0, rows, :], sems.at[len(out_cps)]))
            out_cps[-1].start()
    for c in out_cps:
        c.wait()


@jax.jit
def pallas_parallel_sum__mha_block__dense_activation_mish__prompt_kernel(
    A_x: jax.Array,
    A_wqkv: jax.Array,
    A_wo: jax.Array,
    B_x: jax.Array,
    B_w1: jax.Array,
    B_b1: jax.Array,
    B_w2: jax.Array,
):
    del B_x
    _, S, D = A_x.shape
    F = B_w1.shape[1]
    NF = F // 128
    assert A_x.shape == (1, 2048, H * DH) and NF == 14
    vm = pltpu.VMEM
    hbm = pl.BlockSpec(memory_space=pl.ANY)
    p_shape = vm((S + NGM * 32, TQ), U32)
    return pl.pallas_call(
        _kernel,
        out_shape=jax.ShapeDtypeStruct(A_x.shape, A_x.dtype),
        in_specs=[hbm] * 6,
        out_specs=hbm,
        scratch_shapes=[
            vm((S, D), BF16),
            vm((D, 3 * D), BF16),
            vm((D, D), BF16),
            vm((D, F), BF16),
            vm((F, D), BF16),
            vm((NF, D // 2, 128), U32),
            vm((F // 2, D), U32),
            vm((16, 8, 128), F32),
            vm((S // 2, D), U32),
            vm((D // 128, S // 2, 128), U32),
            vm((D // 128, 2, -(-NGM // 8) * 64, 128), F32),
            vm((H, S // TQ, DH, TQ), F32),
            vm((H, S // TK, 8, TK), U32),
            vm((H, S // TQ, 8, TQ), U32),
            vm((S // 4, 128), U32),
            vm((S // 4, 128), U32),
            vm((S // H // 2, 2048), U32),
            vm((S // TQ, DH, TQ), F32),
            vm((S // TQ, 8, TQ), F32),
            p_shape, p_shape,
            vm((H, S // TQ, 8, TQ), U32),
            vm((S, D), F32),
            vm((S, D), BF16),
            vm((NF, 128), BF16),
            pltpu.SemaphoreType.DMA((16,)),
        ],
        compiler_params=pltpu.CompilerParams(vmem_limit_bytes=100 << 20),
    )(A_x, A_wqkv, A_wo, B_w1, B_b1.reshape(NF, 128), B_w2)
```

```python
import jax
import jax.numpy as jnp
import numpy as np
from jax import lax
from jax.experimental import pallas as pl
from jax.experimental.pallas import tpu as pltpu

F32, BF16, U32 = jnp.float32, jnp.bfloat16, jnp.uint32
LOG2E = float(np.log2(np.e))
H, DH = 32, 16
TQ = 512
TK = 128
NT = TQ // 128
L_LO, L_HI = 2.0 ** -64, 2.0 ** 64

RS = (176, 192)
NGM = max(RS) // 8
V_SPAN = ((0, 1), (0.015, 1.03))
V_RUN = (5, 6)
K_SPAN, K_BATCH = 0.97, 6
CUT = (3, 4)
FFN_START = (1, 0)
PV_LAG = 1
FB = 2
FM = 32
XA, X0 = 256, 768
R1, RB, OL = 128, 256, 128

_reciprocal = getattr(pltpu, "reciprocal", None) or pl.reciprocal


def _pack(x):
    return pltpu.bitcast(x.astype(BF16), U32)


def _unpack(x):
    return pltpu.bitcast(x, BF16)


def _mish(h2):
    e = jnp.exp2(jnp.minimum(h2, 30.0))
    n = e * (e + 2.0)
    return h2 * (n * _reciprocal(n + 2.0, approx=True))


def _kernel(x_hbm, wqkv_hbm, wo_hbm, w1_hbm, b1_hbm, w2_hbm, out_hbm,
           x_v, wqkv_v, wo_v, w1_v, w2_v, w1_s, w2_s, b1_s, xn_s, k_s, kf_s, qt_s, vt_s, qp_s,
           kha_s, khb_s, act_s, oc_s, l_s, pa_s, pb_s, ot_s, acc_s, out_v, b1_v, sems):
    S, D = x_v.shape
    NF = w1_v.shape[1] // 128
    NQB = S // TQ
    SH = S // 2
    NKH = SH // TK
    NP = NQB * NKH
    PR = SH // 2
    FR = S // H
    kh_bufs = (kha_s, khb_s)

    def x_cp(r0, r1, sem):
        return pltpu.make_async_copy(x_hbm.at[0, pl.ds(r0, r1 - r0), :], x_v.at[pl.ds(r0, r1 - r0), :], sems.at[sem])

    def wqkv_cp(i):
        return pltpu.make_async_copy(wqkv_hbm.at[:, pl.ds(i * D, D)], wqkv_v.at[:, pl.ds(i * D, D)], sems.at[2 + i])

    late_cps = [pltpu.make_async_copy(src, dst, sems.at[5 + i])
                for i, (src, dst) in enumerate(((w1_hbm, w1_v), (w2_hbm, w2_v), (wo_hbm, wo_v), (b1_hbm, b1_v)))]

    def kb_slot(d, g):
        i = g * DH + d
        return pl.ds(NQB * PR + (i // NT) * 8, 8), pl.ds((i % NT) * 128, 128)

    def kb_prep(dst, h, kh, d, groups):
        idx = jnp.full((8, 128), ((h % 8) * DH + d) & 127, U32)
        for g in groups:
            kb = jnp.take_along_axis(kf_s[h // 8, kh, pl.ds(g * 8, 8), :], idx, axis=1)
            dst[kb_slot(d, g)] = pltpu.bitcast(kb, U32)

    def kh_prep(h, kh):
        n = (SH - RS[kh]) // 2
        idx = (lax.broadcasted_iota(jnp.int32, (8, 128), 1) % DH + (h % 8) * DH).astype(U32)
        for r in range(0, n, 8):
            k = k_s[h // 8, pl.ds(kh * SH // 2 + r, 8), :]
            kh_bufs[kh][pl.ds(r, 8), :] = jnp.take_along_axis(k, idx, axis=1)

    def pv_dot(h, kh, p_ref, u, j):
        p = _unpack(p_ref[pl.ds(u * PR + j * TK // 2, TK // 2), :])
        return jnp.dot(_unpack(vt_s[h, kh * NKH + j]), p, preferred_element_type=F32)

    def inv_sum(u, l_min, l_max):
        l = jnp.sum(l_s[u], axis=0, keepdims=True)
        r = _reciprocal(l, approx=True)
        return r * (2.0 - l * r), jnp.minimum(l_min, l), jnp.maximum(l_max, l)

    def layernorm(r0, n):
        x = x_v[pl.ds(r0, n), :].astype(F32)
        xc = x - jnp.mean(x, axis=-1, keepdims=True)
        var = jnp.mean(xc * xc, axis=-1, keepdims=True)
        xn_s[pl.ds(r0 // 2, n // 2), :] = _pack(xc * (lax.rsqrt(var + 1e-5) * LOG2E))

    def project(r0, n, i):
        return jnp.dot(_unpack(xn_s[pl.ds(r0 // 2, n // 2), :]), wqkv_v[:, pl.ds(i * D, D)],
                       preferred_element_type=F32)

    def k_proj(r0, n):
        k = project(r0, n, 1)
        kp = _pack(k)
        kh = r0 // SH
        v0 = (kh + 1) * SH - RS[kh]
        lo = max(r0, v0)
        for c in range(D // 128):
            k_s[c, pl.ds(r0 // 2, n // 2), :] = kp[:, c * 128:(c + 1) * 128]
            if lo < r0 + n:
                kf_s[c, kh, pl.ds(lo - v0, r0 + n - lo), :] = k[lo - r0:, c * 128:(c + 1) * 128]

    def qv_proj(r0):
        q = (project(r0, RB, 0) * (DH ** -0.5 / LOG2E)).T
        v = project(r0, RB, 2).T
        u, cols = r0 // TQ, pl.ds(r0 % TQ, RB)
        for h in range(H):
            qt_s[h, u, :, cols] = q[h * DH:(h + 1) * DH]
            qp_s[h, u, :, cols] = _pack(q[h * DH:(h + 1) * DH])
            for t in range(RB // TK):
                vt_s[h, r0 // TK + t] = _pack(v[h * DH:(h + 1) * DH, t * TK:(t + 1) * TK])

    x_cp(0, XA, 0).start()
    wqkv_cp(1).start()
    pb_s[pl.ds(0, NQB * PR), :] = jnp.zeros((NQB * PR, TQ), U32)
    oc_s[...] = jnp.zeros(oc_s.shape, F32)
    ot_s[H - 1] = jnp.zeros(ot_s.shape[1:], U32)
    l_s[...] = jnp.full(l_s.shape, 0.125, F32)
    x_cp(XA, X0, 9).start()
    x_cp(0, XA, 0).wait()
    wqkv_cp(1).wait()
    wqkv_cp(0).start()
    wqkv_cp(2).start()
    for r0 in range(0, XA, R1):
        layernorm(r0, R1)
        if r0 + R1 < XA:
            k_proj(r0, R1)
    x_cp(XA, X0, 9).wait()
    k_proj(XA - R1, R1)
    for r0 in range(XA, X0, R1):
        layernorm(r0, R1)
        if r0 == X0 - 2 * R1:
            x_cp(X0, S, 1).start()
        k_proj(r0, R1)
    wqkv_cp(0).wait()
    wqkv_cp(2).wait()
    for r0 in range(0, X0 - RB, RB):
        qv_proj(r0)
    x_cp(X0, S, 1).wait()
    for c in late_cps:
        c.start()
    qv_proj(X0 - RB)
    for r0 in range(X0, S, R1):
        layernorm(r0, R1)
        if r0 + RB < S:
            k_proj(r0, R1)
    kh_prep(0, 0)
    for d in range(DH):
        kb_prep(pb_s, 0, 0, d, range(RS[0] // 8))
    for r0 in range(X0, S - RB, RB):
        qv_proj(r0)
    for c in late_cps:
        c.wait()
    qv_proj(S - RB)
    k_proj(S - RB, RB)
    for c in range(NF):
        w1_s[c] = pltpu.bitcast(w1_v[:, pl.ds(c * 128, 128)], U32)
    w2_s[...] = pltpu.bitcast(w2_v[...], U32)
    b1 = b1_v[...].astype(F32) * LOG2E
    for c in range(NF):
        b1_s[c] = jnp.broadcast_to(b1[c:c + 1, :], (8, 128))

    ffn_ops = ([(c, r) for r in range(0, FR, FM) for c in range(NF)],
               [op + (r,) for r in range(0, FR, FM) for n in (0, 2)
                for op in ((n, 0), (n, 4), (n, 8), (n, 12), (n + 1, 0), (n + 1, 4), (n + 1, 8))])
    ffn_at = [{lo + i * (NP - lo) // len(ops): op for i, op in enumerate(ops)} for ops, lo in zip(ffn_ops, FFN_START)]
    assert [len(a) for a in ffn_at] == [len(ops) for ops in ffn_ops]

    def score_step(h, kh, l, p_wr, p_rd, h_next, zero, pv_step, ffn_step):
        p_paced = p_wr.at[pl.ds(pl.multiple_of(zero, 16), p_wr.shape[0])]
        kh_prep(h_next, 1 - kh)
        n_mxu = (SH - RS[kh]) // 16
        vpu = sorted(((u, b, t) for u in range(NQB) for t in range(NT) for b in range(RS[kh] // 16)),
                     key=lambda p: (p[0], p[1] // V_RUN[kh], p[2], p[1]))
        ng = RS[1 - kh] // 8
        copies = [(d, range(g, min(g + K_BATCH, ng))) for d in range(DH) for g in range(0, ng, K_BATCH)]
        v0, v1 = V_SPAN[kh]
        events = sorted([((a + 0.5) / (NQB * n_mxu), 0, a) for a in range(NQB * n_mxu)]
                        + [(v0 + (v1 - v0) * (i + 0.5) / len(vpu), 1, i) for i in range(len(vpu))]
                        + [(K_SPAN * (i + 0.5) / len(copies), 2, i) for i in range(len(copies))])

        def add_l(u, t, p):
            for g in (p[:8], p[8:]):
                l[u][t] = g if l[u][t] is None else l[u][t] + g

        def mxu_piece(s, u, a):
            p = jnp.exp2(s)
            for t in range(NT):
                add_l(u, t, p[:, t * 128:(t + 1) * 128])
            p_wr[pl.ds(u * PR + a * 8, 8), :] = _pack(p)

        def vpu_piece(u, b, t):
            s = [None, None]
            for d in range(DH):
                kb = [pltpu.bitcast(p_rd[kb_slot(d, 2 * b + g)], F32) for g in range(2)]
                qd = jnp.broadcast_to(qt_s[h, u, pl.ds(d, 1), pl.ds(t * 128, 128)], (8, 128))
                for g in range(2):
                    s[g] = kb[g] * qd if d == 0 else s[g] + kb[g] * qd
            p = jnp.exp2(jnp.concatenate(s, axis=0))
            add_l(u, t, p)
            p_paced[pl.ds(u * PR + (n_mxu + b) * 8, 8), pl.ds(t * 128, 128)] = _pack(p)

        for period in range(NP):
            u, j = divmod(period, NKH)
            lo, hi = n_mxu * j // NKH, n_mxu * (j + 1) // NKH
            mid = min(lo + CUT[kh], hi) if period in ffn_at[kh] else lo
            for part, (a0, a1) in enumerate(((lo, mid), (mid, hi))):
                if part == 1 and period in ffn_at[kh]:
                    ffn_step(*ffn_at[kh][period])
                if a0 == a1:
                    continue
                k = _unpack(kh_bufs[kh][pl.ds(a0 * 8, (a1 - a0) * 8), :])
                s = jnp.dot(k[:, :DH], _unpack(qp_s[h, u]), preferred_element_type=F32)
                while events and (events[0][1] or events[0][2] < u * n_mxu + a1):
                    _, kind, i = events.pop(0)
                    if kind == 0:
                        a = i - u * n_mxu
                        mxu_piece(s[(a - a0) * 16:(a - a0 + 1) * 16], u, a)
                    elif kind == 1:
                        vpu_piece(*vpu[i])
                    else:
                        kb_prep(p_paced, h_next, 1 - kh, *copies[i])
            if period >= kh * PV_LAG:
                pv_step(*divmod(period - kh * PV_LAG, NKH))
        for period in range(NP - kh * PV_LAG, NP):
            pv_step(*divmod(period, NKH))

    def head(h, carry):
        l_min, l_max = carry
        h_prev, h_next = jnp.maximum(h - 1, 0), jnp.minimum(h + 1, H - 1)
        zero = (h // H) * 16
        inv, live = [], {}
        for u in range(NQB):
            r, l_min, l_max = inv_sum(u, l_min, l_max)
            inv.append(r)

        def pv_prev(u, j):
            live["o"] = (oc_s[u] if j == 0 else live["o"]) + pv_dot(h_prev, 1, pb_s, u, j)
            if j == NKH - 1:
                ot_s[h_prev, u] = _pack(live["o"] * inv[u])

        def pv_this(u, j):
            pv = pv_dot(h, 0, pa_s, u, j)
            live["o"] = pv if j == 0 else live["o"] + pv
            if j == NKH - 1:
                oc_s[u] = live["o"]

        def ffn_up(c, r):
            xn = _unpack(xn_s[pl.ds(pl.multiple_of(h * (FR // 2) + r // 2, 8), FM // 2), :])
            hid = jnp.dot(xn, _unpack(w1_s[c]), preferred_element_type=F32)
            hid = hid + jnp.concatenate([b1_s[c]] * (FM // 8), axis=0)
            act_s[pl.ds(r // 2, FM // 2), pl.ds(c * 128, 128)] = _pack(_mish(hid))

        def ffn_down(n, c, r):
            rows = pl.ds(pl.multiple_of(h * FR + r, FM), FM)
            kt, nt = (2, 2) if c == 12 else (4, 1)
            y = jnp.dot(_unpack(act_s[pl.ds(r // 2, FM // 2), pl.ds(c * 128, kt * 128)]),
                        _unpack(w2_s[pl.ds(c * 64, kt * 64), pl.ds(n * 128, nt * 128)]),
                        preferred_element_type=F32)
            if c == 12:
                acc_s[rows, pl.ds(n * 128, 128)] = live["y"] + y[:, :128]
                live["y"] = y[:, 128:]
            else:
                live["y"] = y if (c == 0 and n % 2 == 0) else live["y"] + y
                if c == 8 and n % 2 == 1:
                    acc_s[rows, pl.ds(n * 128, 128)] = live["y"]

        l = [[None] * NT for _ in range(NQB)]
        score_step(h, 0, l, pa_s, pb_s, h, zero, pv_prev, ffn_up)
        score_step(h, 1, l, pb_s, pa_s, h_next, zero, pv_this, ffn_down)
        for u in range(NQB):
            l_s[u] = jnp.concatenate(l[u], axis=1)
        return l_min, l_max

    one = jnp.ones((1, TQ), F32)
    l_min, l_max = lax.fori_loop(0, H, head, (one, one))
    inv = []
    for u in range(NQB):
        r, l_min, l_max = inv_sum(u, l_min, l_max)
        inv.append(r)

    unsafe = jnp.min(jnp.where((l_min >= L_LO) & (l_max <= L_HI), 1.0, 0.0)) < 0.5

    @pl.when(unsafe)
    def _():
        def shifted_softmax(i, carry):
            h, u = i // NQB, i % NQB
            slot = lax.broadcasted_iota(jnp.int32, (64, TQ), 0) // 8
            q = _unpack(jnp.where(slot == h % 8, jnp.concatenate([qp_s[h, u]] * 8, axis=0), jnp.uint32(0)))

            def scores(j):
                k = _unpack(k_s[h // 8, pl.ds(pl.multiple_of(j * (FB * TK // 2), FB * TK // 2), FB * TK // 2), :])
                return jnp.dot(k, q, preferred_element_type=F32)

            def row_max(j, m):
                return jnp.maximum(m, jnp.max(scores(j), axis=0, keepdims=True))

            m = lax.fori_loop(0, S // (FB * TK), row_max, jnp.full((1, TQ), -jnp.inf, F32))

            def accumulate(j, c):
                p = jnp.exp2(scores(j) - m)
                v = _unpack(jnp.concatenate([vt_s[h, FB * j + i] for i in range(FB)], axis=1))
                return (c[0] + jnp.sum(p, axis=0, keepdims=True),
                        c[1] + jnp.dot(v, p.astype(BF16), preferred_element_type=F32))

            l, o = lax.fori_loop(0, S // (FB * TK), accumulate,
                                 (jnp.zeros((1, TQ), F32), jnp.zeros((DH, TQ), F32)))
            ot_s[h, u] = _pack(o / l)
            return carry

        lax.fori_loop(0, H * NQB, shifted_softmax, 0)

    todo, o_last, out_cps = [(u, j) for u in range(NQB) for j in range(NKH)], {}, []

    def pv_last():
        u, j = todo.pop(0)
        o_last[u] = (oc_s[u] if j == 0 else o_last[u]) + pv_dot(H - 1, 1, pb_s, u, j)
        if j == NKH - 1:
            ot_s[H - 1, u] = jnp.where(unsafe, ot_s[H - 1, u], _pack(o_last[u] * inv[u]))

    for _ in range(NKH):
        pv_last()
    for r0 in range(0, S, RB):
        u, rows = r0 // TQ, pl.ds(r0, RB)
        y = acc_s[rows, :]
        for c in range(D // 128):
            assert not todo or todo[0][0] > u
            ot = jnp.concatenate([ot_s[h, u, :, pl.ds(r0 % TQ, RB)] for h in range(8 * c, 8 * c + 8)], axis=0)
            y = y + lax.dot_general(_unpack(ot), wo_v[pl.ds(c * 128, 128), :], (((0,), (0,)), ((), ())),
                                    preferred_element_type=F32)
            if todo:
                pv_last()
        n = RB if r0 + RB < S else OL
        for r in range(0, RB, n):
            rows = pl.ds(r0 + r, n)
            out_v[rows, :] = (x_v[rows, :].astype(F32) + y[r:r + n] * (1.0 / LOG2E)).astype(out_v.dtype)
            out_cps.append(pltpu.make_async_copy(out_v.at[rows, :], out_hbm.at[0, rows, :], sems.at[len(out_cps)]))
            out_cps[-1].start()
    for c in out_cps:
        c.wait()


@jax.jit
def pallas_parallel_sum__mha_block__dense_activation_mish__prompt_kernel(
    A_x: jax.Array,
    A_wqkv: jax.Array,
    A_wo: jax.Array,
    B_x: jax.Array,
    B_w1: jax.Array,
    B_b1: jax.Array,
    B_w2: jax.Array,
):
    del B_x
    _, S, D = A_x.shape
    F = B_w1.shape[1]
    NF = F // 128
    assert A_x.shape == (1, 2048, H * DH) and NF == 14
    vm = pltpu.VMEM
    hbm = pl.BlockSpec(memory_space=pl.ANY)
    p_shape = vm((S + NGM * 32, TQ), U32)
    return pl.pallas_call(
        _kernel,
        out_shape=jax.ShapeDtypeStruct(A_x.shape, A_x.dtype),
        in_specs=[hbm] * 6,
        out_specs=hbm,
        scratch_shapes=[
            vm((S, D), BF16),
            vm((D, 3 * D), BF16),
            vm((D, D), BF16),
            vm((D, F), BF16),
            vm((F, D), BF16),
            vm((NF, D // 2, 128), U32),
            vm((F // 2, D), U32),
            vm((16, 8, 128), F32),
            vm((S // 2, D), U32),
            vm((D // 128, S // 2, 128), U32),
            vm((D // 128, 2, -(-NGM // 8) * 64, 128), F32),
            vm((H, S // TQ, DH, TQ), F32),
            vm((H, S // TK, 8, TK), U32),
            vm((H, S // TQ, 8, TQ), U32),
            vm((S // 4, 128), U32),
            vm((S // 4, 128), U32),
            vm((S // H // 2, 2048), U32),
            vm((S // TQ, DH, TQ), F32),
            vm((S // TQ, 8, TQ), F32),
            p_shape, p_shape,
            vm((H, S // TQ, 8, TQ), U32),
            vm((S, D), F32),
            vm((S, D), BF16),
            vm((NF, 128), BF16),
            pltpu.SemaphoreType.DMA((16,)),
        ],
        compiler_params=pltpu.CompilerParams(vmem_limit_bytes=100 << 20),
    )(A_x, A_wqkv, A_wo, B_w1, B_b1.reshape(NF, 128), B_w2)
```

```python
import jax
import jax.numpy as jnp
import numpy as np
from jax import lax
from jax.experimental import pallas as pl
from jax.experimental.pallas import tpu as pltpu

F32, BF16, U32 = jnp.float32, jnp.bfloat16, jnp.uint32
LOG2E = float(np.log2(np.e))
H, DH = 32, 16
TQ = 512
TK = 128
NT = TQ // 128
L_LO, L_HI = 2.0 ** -64, 2.0 ** 64

RS = (176, 192)
NGM = max(RS) // 8
V_SPAN = ((0, 1), (0.015, 1.03))
V_RUN = (6, 6)
K_SPAN, K_BATCH = (0.01, 0.97), (6, 7)
M_PHASE = (6, 0)
CUT = (3, 4)
FFN_START = (1, 0)
PV_LAG = 1
FB = 2
FM = 32
XA, X0 = 256, 768
R1, RB, OL = 128, 256, 128

_reciprocal = getattr(pltpu, "reciprocal", None) or pl.reciprocal


def _pack(x):
    return pltpu.bitcast(x.astype(BF16), U32)


def _unpack(x):
    return pltpu.bitcast(x, BF16)


def _mish(h2):
    e = jnp.exp2(jnp.minimum(h2, 30.0))
    n = e * (e + 2.0)
    return h2 * (n * _reciprocal(n + 2.0, approx=True))


def _kernel(x_hbm, wqkv_hbm, wo_hbm, w1_hbm, b1_hbm, w2_hbm, out_hbm,
            x_v, wqkv_v, wo_v, w1_v, w2_v, w1_s, w2_s, b1_s, xn_s, k_s, kf_s, qt_s, vt_s, qp_s,
            kha_s, khb_s, act_s, oc_s, l_s, pa_s, pb_s, ot_s, acc_s, out_v, b1_v, sems):
    S, D = x_v.shape
    NF = w1_v.shape[1] // 128
    NQB = S // TQ
    SH = S // 2
    NKH = SH // TK
    NP = NQB * NKH
    PR = SH // 2
    FR = S // H
    kh_bufs = (kha_s, khb_s)

    def x_cp(r0, r1, sem):
        return pltpu.make_async_copy(x_hbm.at[0, pl.ds(r0, r1 - r0), :], x_v.at[pl.ds(r0, r1 - r0), :], sems.at[sem])

    def wqkv_cp(i):
        return pltpu.make_async_copy(wqkv_hbm.at[:, pl.ds(i * D, D)], wqkv_v.at[:, pl.ds(i * D, D)], sems.at[2 + i])

    late_cps = [pltpu.make_async_copy(src, dst, sems.at[5 + i])
                for i, (src, dst) in enumerate(((w1_hbm, w1_v), (w2_hbm, w2_v), (wo_hbm, wo_v), (b1_hbm, b1_v)))]

    def kb_slot(d, g):
        i = g * DH + d
        return pl.ds(NQB * PR + (i // NT) * 8, 8), pl.ds((i % NT) * 128, 128)

    def kb_prep(dst, h, kh, d, groups):
        idx = jnp.full((8, 128), ((h % 8) * DH + d) & 127, U32)
        for g in groups:
            kb = jnp.take_along_axis(kf_s[h // 8, kh, pl.ds(g * 8, 8), :], idx, axis=1)
            dst[kb_slot(d, g)] = pltpu.bitcast(kb, U32)

    def kh_prep(h, kh):
        n = (SH - RS[kh]) // 2
        idx = (lax.broadcasted_iota(jnp.int32, (8, 128), 1) % DH + (h % 8) * DH).astype(U32)
        for r in range(0, n, 8):
            k = k_s[h // 8, pl.ds(kh * SH // 2 + r, 8), :]
            kh_bufs[kh][pl.ds(r, 8), :] = jnp.take_along_axis(k, idx, axis=1)

    def pv_dot(h, kh, p_ref, u, j):
        p = _unpack(p_ref[pl.ds(u * PR + j * TK // 2, TK // 2), :])
        return jnp.dot(_unpack(vt_s[h, kh * NKH + j]), p, preferred_element_type=F32)

    def inv_sum(u, l_min, l_max):
        l = jnp.sum(l_s[u], axis=0, keepdims=True)
        r = _reciprocal(l, approx=True)
        return r * (2.0 - l * r), jnp.minimum(l_min, l), jnp.maximum(l_max, l)

    def layernorm(r0, n):
        x = x_v[pl.ds(r0, n), :].astype(F32)
        xc = x - jnp.mean(x, axis=-1, keepdims=True)
        var = jnp.mean(xc * xc, axis=-1, keepdims=True)
        xn_s[pl.ds(r0 // 2, n // 2), :] = _pack(xc * (lax.rsqrt(var + 1e-5) * LOG2E))

    def project(r0, n, i):
        return jnp.dot(_unpack(xn_s[pl.ds(r0 // 2, n // 2), :]), wqkv_v[:, pl.ds(i * D, D)],
                       preferred_element_type=F32)

    def k_proj(r0, n):
        k = project(r0, n, 1)
        kp = _pack(k)
        kh = r0 // SH
        v0 = (kh + 1) * SH - RS[kh]
        lo = max(r0, v0)
        for c in range(D // 128):
            k_s[c, pl.ds(r0 // 2, n // 2), :] = kp[:, c * 128:(c + 1) * 128]
            if lo < r0 + n:
                kf_s[c, kh, pl.ds(lo - v0, r0 + n - lo), :] = k[lo - r0:, c * 128:(c + 1) * 128]

    def qv_proj(r0):
        q = (project(r0, RB, 0) * (DH ** -0.5 / LOG2E)).T
        v = project(r0, RB, 2).T
        u, cols = r0 // TQ, pl.ds(r0 % TQ, RB)
        for h in range(H):
            qt_s[h, u, :, cols] = q[h * DH:(h + 1) * DH]
            qp_s[h, u, :, cols] = _pack(q[h * DH:(h + 1) * DH])
            for t in range(RB // TK):
                vt_s[h, r0 // TK + t] = _pack(v[h * DH:(h + 1) * DH, t * TK:(t + 1) * TK])

    x_cp(0, XA, 0).start()
    wqkv_cp(1).start()
    pb_s[pl.ds(0, NQB * PR), :] = jnp.zeros((NQB * PR, TQ), U32)
    oc_s[...] = jnp.zeros(oc_s.shape, F32)
    ot_s[H - 1] = jnp.zeros(ot_s.shape[1:], U32)
    l_s[...] = jnp.full(l_s.shape, 0.125, F32)
    x_cp(XA, X0, 9).start()
    x_cp(0, XA, 0).wait()
    wqkv_cp(1).wait()
    wqkv_cp(0).start()
    wqkv_cp(2).start()
    for r0 in range(0, XA, R1):
        layernorm(r0, R1)
        if r0 + R1 < XA:
            k_proj(r0, R1)
    x_cp(XA, X0, 9).wait()
    k_proj(XA - R1, R1)
    for r0 in range(XA, X0, R1):
        layernorm(r0, R1)
        if r0 == X0 - 2 * R1:
            x_cp(X0, S, 1).start()
        k_proj(r0, R1)
    wqkv_cp(0).wait()
    wqkv_cp(2).wait()
    for r0 in range(0, X0 - RB, RB):
        qv_proj(r0)
    x_cp(X0, S, 1).wait()
    for c in late_cps:
        c.start()
    qv_proj(X0 - RB)
    for r0 in range(X0, S, R1):
        layernorm(r0, R1)
        if r0 + RB < S:
            k_proj(r0, R1)
    kh_prep(0, 0)
    for d in range(DH):
        kb_prep(pb_s, 0, 0, d, range(RS[0] // 8))
    for r0 in range(X0, S - RB, RB):
        qv_proj(r0)
    for c in late_cps:
        c.wait()
    qv_proj(S - RB)
    k_proj(S - RB, RB)
    for c in range(NF):
        w1_s[c] = pltpu.bitcast(w1_v[:, pl.ds(c * 128, 128)], U32)
    w2_s[...] = pltpu.bitcast(w2_v[...], U32)
    b1 = b1_v[...].astype(F32) * LOG2E
    for c in range(NF):
        b1_s[c] = jnp.broadcast_to(b1[c:c + 1, :], (8, 128))

    ffn_ops = ([(c, r) for r in range(0, FR, FM) for c in range(NF)],
               [op + (r,) for r in range(0, FR, FM) for n in (0, 2)
                for op in ((n, 0), (n, 4), (n, 8), (n, 12), (n + 1, 0), (n + 1, 4), (n + 1, 8))])
    ffn_at = [{lo + i * (NP - lo) // len(ops): op for i, op in enumerate(ops)} for ops, lo in zip(ffn_ops, FFN_START)]
    assert [len(a) for a in ffn_at] == [len(ops) for ops in ffn_ops]

    def score_step(h, kh, l, p_wr, p_rd, h_next, zero, pv_step, ffn_step):
        p_paced = p_wr.at[pl.ds(pl.multiple_of(zero, 16), p_wr.shape[0])]
        kh_prep(h_next, 1 - kh)
        n_mxu = (SH - RS[kh]) // 16
        vpu = sorted(((u, b, t) for u in range(NQB) for t in range(NT) for b in range(RS[kh] // 16)),
                     key=lambda p: (p[0], p[1] // V_RUN[kh], p[2] if kh else -p[2], p[1]))
        ng = RS[1 - kh] // 8
        copies = [(d, range(g, min(g + K_BATCH[kh], ng))) for d in range(DH) for g in range(0, ng, K_BATCH[kh])]
        (v0, v1), (k0, k1) = V_SPAN[kh], K_SPAN
        events = sorted([((a + 0.5) / (NQB * n_mxu), 0, a) for a in range(NQB * n_mxu)]
                        + [(v0 + (v1 - v0) * (i + 0.5) / len(vpu), 1, i) for i in range(len(vpu))]
                        + [(k0 + (k1 - k0) * (i + 0.5) / len(copies), 2, i) for i in range(len(copies))])

        def add_l(u, t, p):
            for g in (p[:8], p[8:]):
                l[u][t] = g if l[u][t] is None else l[u][t] + g

        def mxu_piece(s, u, a):
            p = jnp.exp2(s)
            for t in range(NT):
                add_l(u, t, p[:, t * 128:(t + 1) * 128])
            p_wr[pl.ds(u * PR + a * 8, 8), :] = _pack(p)

        def vpu_piece(u, b, t):
            s = [None, None]
            for d in range(DH):
                kb = [pltpu.bitcast(p_rd[kb_slot(d, 2 * b + g)], F32) for g in range(2)]
                qd = jnp.broadcast_to(qt_s[h, u, pl.ds(d, 1), pl.ds(t * 128, 128)], (8, 128))
                for g in range(2):
                    s[g] = kb[g] * qd if d == 0 else s[g] + kb[g] * qd
            p = jnp.exp2(jnp.concatenate(s, axis=0))
            add_l(u, t, p)
            p_paced[pl.ds(u * PR + (n_mxu + b) * 8, 8), pl.ds(t * 128, 128)] = _pack(p)

        for period in range(NP):
            u, j = divmod(period, NKH)
            lo, hi = (n_mxu * j + M_PHASE[kh]) // NKH, (n_mxu * (j + 1) + M_PHASE[kh]) // NKH
            mid = min(lo + CUT[kh], hi) if period in ffn_at[kh] else lo
            for part, (a0, a1) in enumerate(((lo, mid), (mid, hi))):
                if part == 1 and period in ffn_at[kh]:
                    ffn_step(*ffn_at[kh][period])
                if a0 == a1:
                    continue
                k = _unpack(kh_bufs[kh][pl.ds(a0 * 8, (a1 - a0) * 8), :])
                s = jnp.dot(k[:, :DH], _unpack(qp_s[h, u]), preferred_element_type=F32)
                while events and (events[0][1] or events[0][2] < u * n_mxu + a1):
                    _, kind, i = events.pop(0)
                    if kind == 0:
                        a = i - u * n_mxu
                        mxu_piece(s[(a - a0) * 16:(a - a0 + 1) * 16], u, a)
                    elif kind == 1:
                        vpu_piece(*vpu[i])
                    else:
                        kb_prep(p_paced, h_next, 1 - kh, *copies[i])
            if period >= kh * PV_LAG:
                pv_step(*divmod(period - kh * PV_LAG, NKH))
        for period in range(NP - kh * PV_LAG, NP):
            pv_step(*divmod(period, NKH))

    def head(h, carry):
        l_min, l_max = carry
        h_prev, h_next = jnp.maximum(h - 1, 0), jnp.minimum(h + 1, H - 1)
        zero = (h // H) * 16
        inv, live = [], {}
        for u in range(NQB):
            r, l_min, l_max = inv_sum(u, l_min, l_max)
            inv.append(r)

        def pv_prev(u, j):
            live["o"] = (oc_s[u] if j == 0 else live["o"]) + pv_dot(h_prev, 1, pb_s, u, j)
            if j == NKH - 1:
                ot_s[h_prev, u] = _pack(live["o"] * inv[u])

        def pv_this(u, j):
            pv = pv_dot(h, 0, pa_s, u, j)
            live["o"] = pv if j == 0 else live["o"] + pv
            if j == NKH - 1:
                oc_s[u] = live["o"]

        def ffn_up(c, r):
            xn = _unpack(xn_s[pl.ds(pl.multiple_of(h * (FR // 2) + r // 2, 8), FM // 2), :])
            hid = jnp.dot(xn, _unpack(w1_s[c]), preferred_element_type=F32)
            hid = hid + jnp.concatenate([b1_s[c]] * (FM // 8), axis=0)
            act_s[pl.ds(r // 2, FM // 2), pl.ds(c * 128, 128)] = _pack(_mish(hid))

        def ffn_down(n, c, r):
            rows = pl.ds(pl.multiple_of(h * FR + r, FM), FM)
            kt, nt = (2, 2) if c == 12 else (4, 1)
            y = jnp.dot(_unpack(act_s[pl.ds(r // 2, FM // 2), pl.ds(c * 128, kt * 128)]),
                        _unpack(w2_s[pl.ds(c * 64, kt * 64), pl.ds(n * 128, nt * 128)]),
                        preferred_element_type=F32)
            if c == 12:
                acc_s[rows, pl.ds(n * 128, 128)] = live["y"] + y[:, :128]
                live["y"] = y[:, 128:]
            else:
                live["y"] = y if (c == 0 and n % 2 == 0) else live["y"] + y
                if c == 8 and n % 2 == 1:
                    acc_s[rows, pl.ds(n * 128, 128)] = live["y"]

        l = [[None] * NT for _ in range(NQB)]
        score_step(h, 0, l, pa_s, pb_s, h, zero, pv_prev, ffn_up)
        score_step(h, 1, l, pb_s, pa_s, h_next, zero, pv_this, ffn_down)
        for u in range(NQB):
            l_s[u] = jnp.concatenate(l[u], axis=1)
        return l_min, l_max

    one = jnp.ones((1, TQ), F32)
    l_min, l_max = lax.fori_loop(0, H, head, (one, one))
    inv = []
    for u in range(NQB):
        r, l_min, l_max = inv_sum(u, l_min, l_max)
        inv.append(r)

    unsafe = jnp.min(jnp.where((l_min >= L_LO) & (l_max <= L_HI), 1.0, 0.0)) < 0.5

    @pl.when(unsafe)
    def _():
        def shifted_softmax(i, carry):
            h, u = i // NQB, i % NQB
            slot = lax.broadcasted_iota(jnp.int32, (64, TQ), 0) // 8
            q = _unpack(jnp.where(slot == h % 8, jnp.concatenate([qp_s[h, u]] * 8, axis=0), np.uint32(0)))

            def scores(j):
                k = _unpack(k_s[h // 8, pl.ds(pl.multiple_of(j * (FB * TK // 2), FB * TK // 2), FB * TK // 2), :])
                return jnp.dot(k, q, preferred_element_type=F32)

            def row_max(j, m):
                return jnp.maximum(m, jnp.max(scores(j), axis=0, keepdims=True))

            m = lax.fori_loop(0, S // (FB * TK), row_max, jnp.full((1, TQ), -jnp.inf, F32))

            def accumulate(j, c):
                p = jnp.exp2(scores(j) - m)
                v = _unpack(jnp.concatenate([vt_s[h, FB * j + i] for i in range(FB)], axis=1))
                return (c[0] + jnp.sum(p, axis=0, keepdims=True),
                        c[1] + jnp.dot(v, p.astype(BF16), preferred_element_type=F32))

            l, o = lax.fori_loop(0, S // (FB * TK), accumulate,
                                 (jnp.zeros((1, TQ), F32), jnp.zeros((DH, TQ), F32)))
            ot_s[h, u] = _pack(o / l)
            return carry

        lax.fori_loop(0, H * NQB, shifted_softmax, 0)

    todo, o_last, out_cps = [(u, j) for u in range(NQB) for j in range(NKH)], {}, []

    def pv_last():
        u, j = todo.pop(0)
        o_last[u] = (oc_s[u] if j == 0 else o_last[u]) + pv_dot(H - 1, 1, pb_s, u, j)
        if j == NKH - 1:
            ot_s[H - 1, u] = jnp.where(unsafe, ot_s[H - 1, u], _pack(o_last[u] * inv[u]))

    for _ in range(NKH):
        pv_last()
    for r0 in range(0, S, RB):
        u, rows = r0 // TQ, pl.ds(r0, RB)
        y = acc_s[rows, :]
        for c in range(D // 128):
            assert not todo or todo[0][0] > u
            ot = jnp.concatenate([ot_s[h, u, :, pl.ds(r0 % TQ, RB)] for h in range(8 * c, 8 * c + 8)], axis=0)
            y = y + lax.dot_general(_unpack(ot), wo_v[pl.ds(c * 128, 128), :], (((0,), (0,)), ((), ())),
                                    preferred_element_type=F32)
            if todo:
                pv_last()
        n = RB if r0 + RB < S else OL
        for r in range(0, RB, n):
            rows = pl.ds(r0 + r, n)
            out_v[rows, :] = (x_v[rows, :].astype(F32) + y[r:r + n] * (1.0 / LOG2E)).astype(out_v.dtype)
            out_cps.append(pltpu.make_async_copy(out_v.at[rows, :], out_hbm.at[0, rows, :], sems.at[len(out_cps)]))
            out_cps[-1].start()
    for c in out_cps:
        c.wait()


@jax.jit
def pallas_parallel_sum__mha_block__dense_activation_mish__prompt_kernel(
    A_x: jax.Array,
    A_wqkv: jax.Array,
    A_wo: jax.Array,
    B_x: jax.Array,
    B_w1: jax.Array,
    B_b1: jax.Array,
    B_w2: jax.Array,
):
    del B_x
    _, S, D = A_x.shape
    F = B_w1.shape[1]
    NF = F // 128
    assert A_x.shape == (1, 2048, H * DH) and NF == 14
    vm = pltpu.VMEM
    hbm = pl.BlockSpec(memory_space=pl.ANY)
    p_shape = vm((S + NGM * 32, TQ), U32)
    return pl.pallas_call(
        _kernel,
        out_shape=jax.ShapeDtypeStruct(A_x.shape, A_x.dtype),
        in_specs=[hbm] * 6,
        out_specs=hbm,
        scratch_shapes=[
            vm((S, D), BF16),
            vm((D, 3 * D), BF16),
            vm((D, D), BF16),
            vm((D, F), BF16),
            vm((F, D), BF16),
            vm((NF, D // 2, 128), U32),
            vm((F // 2, D), U32),
            vm((16, 8, 128), F32),
            vm((S // 2, D), U32),
            vm((D // 128, S // 2, 128), U32),
            vm((D // 128, 2, -(-NGM // 8) * 64, 128), F32),
            vm((H, S // TQ, DH, TQ), F32),
            vm((H, S // TK, 8, TK), U32),
            vm((H, S // TQ, 8, TQ), U32),
            vm((S // 4, 128), U32),
            vm((S // 4, 128), U32),
            vm((S // H // 2, 2048), U32),
            vm((S // TQ, DH, TQ), F32),
            vm((S // TQ, 8, TQ), F32),
            p_shape, p_shape,
            vm((H, S // TQ, 8, TQ), U32),
            vm((S, D), F32),
            vm((S, D), BF16),
            vm((NF, 128), BF16),
            pltpu.SemaphoreType.DMA((16,)),
        ],
        compiler_params=pltpu.CompilerParams(vmem_limit_bytes=100 << 20),
    )(A_x, A_wqkv, A_wo, B_w1, B_b1.reshape(NF, 128), B_w2)
```
